```python
import jax
import jax.numpy as jnp

def _softmax(x, axis=-1):
    return jax.nn.softmax(x, axis=axis)

def _gelu(x):
    return jax.nn.gelu(x, approximate=True)

def _silu(x):
    return jax.nn.silu(x)

def _sigmoid(x):
    return jax.nn.sigmoid(x)

def _layernorm(x, axis=-1, eps=1e-05):
    m = jnp.mean(x, axis=axis, keepdims=True)
    v = jnp.var(x, axis=axis, keepdims=True)
    return (x - m) / jnp.sqrt(v + eps)

def _scatter_add(tgt, idx, src, axis=0):
    return tgt.at[idx].add(src)

def _segment_sum(src, seg, n):
    return jax.ops.segment_sum(src, seg, n)

class _Rng:

    def __init__(self, key):
        self._k = key

    def _next(self):
        self._k, sub = jax.random.split(self._k)
        return sub

    def normal(self, shape):
        return jax.random.normal(self._next(), shape, dtype=jnp.bfloat16)

    def randint(self, lo, hi, shape):
        return jax.random.randint(self._next(), shape, lo, hi, dtype=jnp.int32)

    def uniform(self, shape, lo=0.0, hi=1.0):
        return jax.random.uniform(self._next(), shape, jnp.bfloat16, lo, hi)

    def permutation(self, n):
        return jax.random.permutation(self._next(), n)
kernel_name = 'adaLN_cond__compressed_kv_cla__glu_gated_geglu__decode'

def setup_inputs():
    _rng = _Rng(jax.random.key(int.from_bytes(__import__("os").urandom(4), "little")))
    _w = lambda a: (lambda t: t.astype(jnp.bfloat16) if jnp.issubdtype(t.dtype, jnp.floating) else t)(jnp.asarray(a))

    def _A_setup():
        B, H, Sq, Sk, D, M = (1, 32, 1, 32768, 128, 512)
        Dc = 4 * D
        return {'x': _w((lambda *s: _rng.normal(s) * 0.05)(B, Sq, M)), 'c_kv': _w((lambda *s: _rng.normal(s) * 0.05)(B, Sk, Dc)), 'w_q': _w((lambda *s: _rng.normal(s) * 0.05)(M, H, D) * M ** (-0.5)), 'w_uk': _w((lambda *s: _rng.normal(s) * 0.05)(Dc, H, D) * Dc ** (-0.5)), 'w_uv': _w((lambda *s: _rng.normal(s) * 0.05)(Dc, H, D) * Dc ** (-0.5)), 'w_o': _w((lambda *s: _rng.normal(s) * 0.05)(H, D, M) * (H * D) ** (-0.5))}
    _A_in = _A_setup()

    def _B_setup():
        B, S, Dm, Df = (1, 1, 512, 1792)
        return {'x': _w((lambda *s: _rng.normal(s) * 0.05)(B, S, Dm)), 'w_gate': _w((lambda *s: _rng.normal(s) * 0.05)(Dm, Df) * Dm ** (-0.5)), 'w_up': _w((lambda *s: _rng.normal(s) * 0.05)(Dm, Df) * Dm ** (-0.5)), 'w_down': _w((lambda *s: _rng.normal(s) * 0.05)(Df, Dm) * Df ** (-0.5))}
    _B_in = _B_setup()
    return {'A_x': _A_in['x'], 'A_c_kv': _A_in['c_kv'], 'A_w_q': _A_in['w_q'], 'A_w_uk': _A_in['w_uk'], 'A_w_uv': _A_in['w_uv'], 'A_w_o': _A_in['w_o'], 'B_x': _B_in['x'], 'B_w_gate': _B_in['w_gate'], 'B_w_up': _B_in['w_up'], 'B_w_down': _B_in['w_down'], 'c': _w((lambda *s: _rng.normal(s) * 0.05)(1, 512)), 'w_mod': _w((lambda *s: _rng.normal(s) * 0.05)(512, 6 * 512) * 512 ** (-0.5))}

def reference(A_x, A_c_kv, A_w_q, A_w_uk, A_w_uv, A_w_o, B_x, B_w_gate, B_w_up, B_w_down, c, w_mod):

    def _A_ref(x, c_kv, w_q, w_uk, w_uv, w_o):
        B, Sq, M = (x.shape[0], x.shape[1], x.shape[2])
        Sk = c_kv.shape[1]
        H, D = (w_q.shape[1], w_q.shape[2])
        q = jnp.einsum('bqm,mhd->bhqd', x, w_q)
        k = jnp.einsum('bkc,chd->bhkd', c_kv, w_uk)
        v = jnp.einsum('bkc,chd->bhkd', c_kv, w_uv)
        scores = jnp.einsum('bhqd,bhkd->bhqk', q, k) * D ** (-0.5)
        off = Sk - Sq
        qi = jnp.arange(Sq)[:, None]
        kj = jnp.arange(Sk)[None, :]
        cmask = kj <= qi + off
        scores = jnp.where(cmask[None, None], scores, -1000000000.0)
        p = _softmax(scores, axis=-1)
        ctx = jnp.einsum('bhqk,bhkd->bhqd', p, v)
        return jnp.einsum('bhqd,hdm->bqm', ctx, w_o)

    def _B_ref(x, w_gate, w_up, w_down):
        g = jnp.einsum('bsd,df->bsf', x, w_gate)
        u = jnp.einsum('bsd,df->bsf', x, w_up)
        h = _gelu(g) * u
        return jnp.einsum('bsf,fd->bsd', h, w_down)
    x = A_x
    mod = (_silu(c) @ w_mod).reshape(c.shape[0], 6, 1, -1)
    sa, ca, ga, sb, cb, gb = (mod[:, 0].copy(), mod[:, 1].copy(), mod[:, 2].copy(), mod[:, 3].copy(), mod[:, 4].copy(), mod[:, 5].copy())
    h = _layernorm(x, axis=-1) * (1 + ca) + sa
    x = x + ga * _A_ref(h, A_c_kv, A_w_q, A_w_uk, A_w_uv, A_w_o)
    h = _layernorm(x, axis=-1) * (1 + cb) + sb
    x = x + gb * _B_ref(h, B_w_gate, B_w_up, B_w_down)
    return x
```

```python
import math

import jax
import jax.numpy as jnp
import jax.experimental.pallas as pl
import jax.experimental.pallas.tpu as pltpu


F32 = jnp.float32
BF16 = jnp.bfloat16
EPS = 1e-5
NT = (((1,), (1,)), ((), ()))

KV_CHUNK = 2048
KV_SUB = 512
WIN = 3


def _ln(x):
    m = jnp.mean(x, axis=-1, keepdims=True)
    d = x - m
    v = jnp.mean(d * d, axis=-1, keepdims=True)
    return d * jax.lax.rsqrt(v + EPS)


def _gelu(x):
    k = math.sqrt(2.0 / math.pi)
    return 0.5 * x * (1.0 + jnp.tanh(k * (x + 0.044715 * (x * x * x))))


@jax.jit
def pallas_adaLN_cond__compressed_kv_cla__glu_gated_geglu__decode_kernel(
    A_x: jax.Array,
    A_c_kv: jax.Array,
    A_w_q: jax.Array,
    A_w_uk: jax.Array,
    A_w_uv: jax.Array,
    A_w_o: jax.Array,
    B_x: jax.Array,
    B_w_gate: jax.Array,
    B_w_up: jax.Array,
    B_w_down: jax.Array,
    c: jax.Array,
    w_mod: jax.Array,
):
    del B_x
    _, Sq, M = A_x.shape
    _, Sk, Dc = A_c_kv.shape
    _, H, D = A_w_q.shape
    Df = B_w_gate.shape[1]
    assert (Sq, H, D) == (1, 32, 128) and M % 128 == 0 and Dc % 128 == 0
    assert Sk % KV_CHUNK == 0 and KV_CHUNK % KV_SUB == 0
    NCK = Sk // KV_CHUNK
    NB_M, NB_C = M // 128, Dc // 128
    RB = 128 * H
    NWO = 4
    WD_SPLITS = (0, 768, 1536, Df)
    scale = float(D) ** -0.5 * math.log2(math.e)

    def kernel(x_hbm, ckv_hbm, wq_hbm, wuk_hbm, wuv_hbm, wo_hbm, wg_hbm, wu_hbm, wd_hbm,
               c_hbm, wmod_hbm, o_ref,
               x_v, c_v, wmod_v, wq_v, wuk_v, ckv_v, wuv_v, wo_v, wg_v, wu_v, wd_v,
               e_v, l_v, q_v, sem, sem_kv):
        def cp(src, dst, i):
            return pltpu.make_async_copy(src, dst, sem.at[i])

        def kv_copy(i):
            rows = pl.ds(i * KV_CHUNK if isinstance(i, int) else pl.multiple_of(i * KV_CHUNK, KV_CHUNK), KV_CHUNK)
            return pltpu.make_async_copy(ckv_hbm.at[rows], ckv_v.at[rows], sem_kv.at[i])

        cp_wmod = cp(wmod_hbm, wmod_v, 0)
        cp_c = cp(c_hbm, c_v, 1)
        cp_x = cp(x_hbm, x_v, 2)
        cp_wq = cp(wq_hbm, wq_v, 3)
        cp_wuk = cp(wuk_hbm, wuk_v, 4)
        cp_wuv = [cp(wuv_hbm.at[pl.ds(b * RB, RB)], wuv_v.at[pl.ds(b * RB, RB)], 5 + b)
                  for b in range(NB_C)]
        ro = H * D // NWO
        cp_wo = [cp(wo_hbm.at[pl.ds(b * ro, ro)], wo_v.at[pl.ds(b * ro, ro)], 5 + NB_C + b)
                 for b in range(NWO)]
        n0 = 5 + NB_C + NWO
        cp_wg = cp(wg_hbm, wg_v, n0)
        cp_wu = cp(wu_hbm, wu_v, n0 + 1)
        cp_wd = [cp(wd_hbm.at[pl.ds(a, b - a)], wd_v.at[pl.ds(a, b - a)], n0 + 2 + i)
                 for i, (a, b) in enumerate(zip(WD_SPLITS[:-1], WD_SPLITS[1:]))]

        head = [cp_wmod, cp_wq, cp_wuk]
        tail = cp_wuv + cp_wo + [cp_wg, cp_wu] + cp_wd

        def start_nth(n):
            if n < len(head):
                head[n].start()
            elif n < len(head) + NCK:
                kv_copy(n - len(head)).start()
            elif n < len(head) + NCK + len(tail):
                tail[n - len(head) - NCK].start()

        def wait_nth(n, d):
            d.wait()
            start_nth(n + WIN)

        start_nth(0)
        cp_c.start()
        cp_x.start()
        for n in range(1, WIN):
            start_nth(n)

        r_i = jax.lax.broadcasted_iota(jnp.int32, (128, RB), 0)
        n_i = jax.lax.broadcasted_iota(jnp.int32, (128, RB), 1)
        e_v[...] = jnp.where(r_i == n_i // H, 1.0, 0.0).astype(BF16)

        def diag_mask(rows):
            rr = jax.lax.broadcasted_iota(jnp.int32, (rows, RB), 0)
            nn = jax.lax.broadcasted_iota(jnp.int32, (rows, RB), 1)
            return (rr % H) == (nn % H)

        cp_c.wait()
        cp_x.wait()
        cf = c_v[...].astype(F32)
        sc = (cf * jax.nn.sigmoid(cf)).astype(BF16)
        wait_nth(0, cp_wmod)
        mod = jnp.dot(sc, wmod_v[...], preferred_element_type=F32)
        sa, ca, ga, sb, cb, gb = [mod[:, i * M:(i + 1) * M] for i in range(6)]
        x = x_v[0].astype(F32)
        h = (_ln(x) * (1.0 + ca) + sa).astype(BF16)

        hrep = jnp.dot(
            jnp.concatenate([h[:, b * 128:(b + 1) * 128] for b in range(NB_M)], axis=0),
            e_v[...], preferred_element_type=F32)
        wait_nth(1, cp_wq)
        q = jnp.zeros((H, D), F32)
        for b in range(NB_M):
            lq = jnp.where(diag_mask(H), hrep[b:b + 1, :], 0.0).astype(BF16)
            q = q + jnp.dot(lq, wq_v[b * RB:(b + 1) * RB, :], preferred_element_type=F32)
        qb = q.astype(BF16)

        wait_nth(2, cp_wuk)
        qa = []
        for b in range(NB_C):
            r = jax.lax.dot_general(qb, wuk_v[b * RB:(b + 1) * RB, :], NT,
                                    preferred_element_type=F32)
            rm = jnp.where(diag_mask(H), r * scale, 0.0).astype(BF16)
            qa.append(jax.lax.dot_general(rm, e_v[...], NT, preferred_element_type=F32))
        q_v[...] = jnp.concatenate(qa, axis=1).astype(BF16)

        def kv_body(i, carry):
            m_prev, l_prev, acc = carry
            kv_copy(i).wait()

            @pl.when(i + WIN < NCK)
            def _():
                kv_copy(i + WIN).start()

            for t in range(WIN):
                @pl.when(i + WIN == NCK + t)
                def _():
                    tail[t].start()
            qabs = q_v[...]
            for j in range(KV_CHUNK // KV_SUB):
                rows = pl.ds(pl.multiple_of(i * KV_CHUNK + j * KV_SUB, KV_SUB), KV_SUB)
                ck = ckv_v[rows, :]
                s = jax.lax.dot_general(qabs, ck, NT, preferred_element_type=F32)
                m_new = jnp.maximum(m_prev, jnp.max(s, axis=1, keepdims=True))
                alpha = jnp.exp2(m_prev - m_new)
                p = jnp.exp2(s - m_new)
                l_prev = l_prev * alpha + jnp.sum(p, axis=1, keepdims=True)
                acc = acc * alpha + jnp.dot(p.astype(BF16), ck, preferred_element_type=F32)
                m_prev = m_new
            return m_prev, l_prev, acc

        m0 = jnp.full((H, 1), -1e30, F32)
        l0 = jnp.zeros((H, 1), F32)
        a0 = jnp.zeros((H, Dc), F32)
        _, l_fin, acc = jax.lax.fori_loop(0, NCK, kv_body, (m0, l0, a0))
        o_lat = (acc / l_fin).astype(BF16)

        orep = jnp.dot(
            jnp.concatenate([o_lat[:, b * 128:(b + 1) * 128] for b in range(NB_C)], axis=0),
            e_v[...], preferred_element_type=F32)
        l_v[...] = jnp.where(diag_mask(NB_C * H), orep, 0.0).astype(BF16)
        ctx = jnp.zeros((H, D), F32)
        for b in range(NB_C):
            wait_nth(3 + NCK + b, cp_wuv[b])
            ctx = ctx + jnp.dot(l_v[b * H:(b + 1) * H, :], wuv_v[b * RB:(b + 1) * RB, :],
                                preferred_element_type=F32)

        rowd = jax.lax.broadcasted_iota(jnp.int32, (H, D), 0)
        att = jnp.zeros((H, M), F32)
        hpp = H // NWO
        for b in range(NWO):
            lo = jnp.concatenate(
                [jnp.where(rowd == b * hpp + j, ctx, 0.0) for j in range(hpp)], axis=1
            ).astype(BF16)
            wait_nth(3 + NCK + NB_C + b, cp_wo[b])
            att = att + jnp.dot(lo, wo_v[b * ro:(b + 1) * ro, :], preferred_element_type=F32)
        x1 = x + ga * jnp.sum(att, axis=0, keepdims=True)

        h2 = (_ln(x1) * (1.0 + cb) + sb).astype(BF16)
        wait_nth(3 + NCK + NB_C + NWO, cp_wg)
        g = jnp.dot(h2, wg_v[...], preferred_element_type=F32)
        wait_nth(3 + NCK + NB_C + NWO + 1, cp_wu)
        u = jnp.dot(h2, wu_v[...], preferred_element_type=F32)
        act = (_gelu(g) * u).astype(BF16)
        ffn = jnp.zeros((1, M), F32)
        for i, (a, b) in enumerate(zip(WD_SPLITS[:-1], WD_SPLITS[1:])):
            wait_nth(3 + NCK + NB_C + NWO + 2 + i, cp_wd[i])
            ffn = ffn + jnp.dot(act[:, a:b], wd_v[a:b, :], preferred_element_type=F32)
        o_ref[0] = (x1 + gb * ffn).astype(o_ref.dtype)

    hbm = pl.BlockSpec(memory_space=pl.ANY)
    n_sem = 5 + NB_C + NWO + 2 + len(WD_SPLITS) - 1
    return pl.pallas_call(
        kernel,
        in_specs=[hbm] * 11,
        out_specs=pl.BlockSpec(memory_space=pltpu.VMEM),
        out_shape=jax.ShapeDtypeStruct((1, Sq, M), A_x.dtype),
        scratch_shapes=[
            pltpu.VMEM((1, Sq, M), BF16),
            pltpu.VMEM((1, M), BF16),
            pltpu.VMEM((M, 6 * M), BF16),
            pltpu.VMEM((M * H, D), BF16),
            pltpu.VMEM((Dc * H, D), BF16),
            pltpu.VMEM((Sk, Dc), BF16),
            pltpu.VMEM((Dc * H, D), BF16),
            pltpu.VMEM((H * D, M), BF16),
            pltpu.VMEM((M, Df), BF16),
            pltpu.VMEM((M, Df), BF16),
            pltpu.VMEM((Df, M), BF16),
            pltpu.VMEM((128, RB), BF16),
            pltpu.VMEM((NB_C * H, RB), BF16),
            pltpu.VMEM((H, Dc), BF16),
            pltpu.SemaphoreType.DMA((n_sem,)),
            pltpu.SemaphoreType.DMA((NCK,)),
        ],
        compiler_params=pltpu.CompilerParams(vmem_limit_bytes=100 * 1024 * 1024),
    )(
        A_x, A_c_kv.reshape(Sk, Dc), A_w_q.reshape(M * H, D), A_w_uk.reshape(Dc * H, D),
        A_w_uv.reshape(Dc * H, D), A_w_o.reshape(H * D, M), B_w_gate, B_w_up, B_w_down,
        c, w_mod,
    )
```

```python
import math

import jax
import jax.numpy as jnp
import jax.experimental.pallas as pl
import jax.experimental.pallas.tpu as pltpu


F32 = jnp.float32
BF16 = jnp.bfloat16
EPS = 1e-5
NT = (((1,), (1,)), ((), ()))

KV_DMA = 4096
KV_STEP = 1024
WD_STEP = 256
WD_DMAS = (0, 1024, 1536, 1792)
WIN = 3


def _ln(x):
    m = jnp.mean(x, axis=-1, keepdims=True)
    d = x - m
    v = jnp.mean(d * d, axis=-1, keepdims=True)
    return d * jax.lax.rsqrt(v + EPS)


def _gelu(x):
    k = math.sqrt(2.0 / math.pi)
    return 0.5 * x * (1.0 + jnp.tanh(k * (x + 0.044715 * (x * x * x))))


@jax.jit
def pallas_adaLN_cond__compressed_kv_cla__glu_gated_geglu__decode_kernel(
    A_x: jax.Array,
    A_c_kv: jax.Array,
    A_w_q: jax.Array,
    A_w_uk: jax.Array,
    A_w_uv: jax.Array,
    A_w_o: jax.Array,
    B_x: jax.Array,
    B_w_gate: jax.Array,
    B_w_up: jax.Array,
    B_w_down: jax.Array,
    c: jax.Array,
    w_mod: jax.Array,
):
    del B_x
    _, Sq, M = A_x.shape
    _, Sk, Dc = A_c_kv.shape
    _, H, D = A_w_q.shape
    Df = B_w_gate.shape[1]
    assert (Sq, H, D) == (1, 32, 128) and M == Dc and M % 128 == 0
    assert Sk % KV_DMA == 0 and KV_DMA % KV_STEP == 0
    assert Df == WD_DMAS[-1] and all(b % WD_STEP == 0 for b in WD_DMAS)
    NKV = Sk // KV_DMA
    NB = M // 128
    RB = 128 * H
    HPB = 8
    scale = float(D) ** -0.5 * math.log2(math.e)

    def kernel(x_hbm, ckv_hbm, wq_hbm, wuk_hbm, wuv_hbm, wo_hbm, wg_hbm, wu_hbm, wd_hbm,
               c_hbm, wmod_hbm, o_ref,
               x_v, c_v, wmod_v, wq_v, wuk_v, ckv_v, wuv_v, wo_v, wgu_v, wd_v,
               e_v, a_v, q_v, gu_v, act_v, sem):
        pairs = [(wmod_hbm, wmod_v), (wq_hbm, wq_v), (wuk_hbm, wuk_v)]
        N_KV0 = len(pairs)
        pairs += [(ckv_hbm.at[pl.ds(i * KV_DMA, KV_DMA)], ckv_v.at[pl.ds(i * KV_DMA, KV_DMA)])
                  for i in range(NKV)]
        N_UV = len(pairs)
        pairs += [(wuv_hbm, wuv_v), (wo_hbm, wo_v), (wg_hbm, wgu_v.at[0]), (wu_hbm, wgu_v.at[1])]
        N_WD = len(pairs)
        pairs += [(wd_hbm.at[pl.ds(a, b - a)], wd_v.at[pl.ds(a, b - a)])
                  for a, b in zip(WD_DMAS[:-1], WD_DMAS[1:])]

        def copy(n):
            return pltpu.make_async_copy(pairs[n][0], pairs[n][1], sem.at[n % WIN])

        def start(n):
            if n < len(pairs):
                copy(n).start()

        def wait(n):
            copy(n).wait()
            start(n + WIN)

        def kv_copy(i):
            rows = pl.ds(pl.multiple_of(i * KV_DMA, KV_DMA), KV_DMA)
            return pltpu.make_async_copy(ckv_hbm.at[rows], ckv_v.at[rows],
                                         sem.at[(N_KV0 + i) % WIN])

        cp_c = pltpu.make_async_copy(c_hbm, c_v, sem.at[0])
        cp_x = pltpu.make_async_copy(x_hbm, x_v, sem.at[0])
        start(0)
        cp_c.start()
        cp_x.start()
        for n in range(1, WIN):
            start(n)

        r_i = jax.lax.broadcasted_iota(jnp.int32, (128, RB), 0)
        n_i = jax.lax.broadcasted_iota(jnp.int32, (128, RB), 1)
        e_v[...] = jnp.where(r_i == n_i // H, 1.0, 0.0).astype(BF16)

        row_h = jax.lax.broadcasted_iota(jnp.int32, (H, 128), 0)
        diag = row_h == (jax.lax.broadcasted_iota(jnp.int32, (H, 128), 1) % H)

        def keep_diag(r):
            return jnp.concatenate(
                [jnp.where(diag, r[:, t * 128:(t + 1) * 128], 0.0) for t in range(RB // 128)],
                axis=1).astype(BF16)

        def head_proj(w_v):
            def body(b, out):
                rep = jnp.dot(a_v[b], e_v[...], preferred_element_type=F32)
                rows = pl.ds(pl.multiple_of(b * RB, RB), RB)
                return out + jnp.dot(keep_diag(rep), w_v[rows, :], preferred_element_type=F32)
            return jax.lax.fori_loop(0, NB, body, jnp.zeros((H, D), F32))

        copy(0).wait()
        cp_c.wait()
        cp_x.wait()
        start(WIN)
        cf = c_v[...].astype(F32)
        sc = (cf * jax.nn.sigmoid(cf)).astype(BF16)
        mod = jnp.dot(sc, wmod_v[...], preferred_element_type=F32)
        sa, ca, ga, sb, cb, gb = [mod[:, i * M:(i + 1) * M] for i in range(6)]
        x = x_v[0].astype(F32)
        h = _ln(x) * (1.0 + ca) + sa

        for b in range(NB):
            a_v[b] = jnp.broadcast_to(h[:, b * 128:(b + 1) * 128], (H, 128)).astype(BF16)
        wait(1)
        qb = head_proj(wq_v).astype(BF16)

        wait(2)

        def uk_body(b, _):
            rows = pl.ds(pl.multiple_of(b * RB, RB), RB)
            r = jax.lax.dot_general(qb, wuk_v[rows, :], NT, preferred_element_type=F32)
            qa = jax.lax.dot_general(keep_diag(r * scale), e_v[...], NT,
                                     preferred_element_type=F32)
            a_v[b] = qa.astype(BF16)
            return 0
        jax.lax.fori_loop(0, NB, uk_body, 0)
        q_v[...] = jnp.concatenate([a_v[b] for b in range(NB)], axis=1)

        SPD = KV_DMA // KV_STEP

        def kv_body(j, carry):
            m_prev, l_prev, acc = carry

            @pl.when(j % SPD == 0)
            def _():
                i = j // SPD
                kv_copy(i).wait()

                @pl.when(i + WIN < NKV)
                def _():
                    kv_copy(i + WIN).start()

                for t in range(WIN):
                    @pl.when(i + WIN == NKV + t)
                    def _():
                        start(N_UV + t)

            ck = ckv_v[pl.ds(pl.multiple_of(j * KV_STEP, KV_STEP), KV_STEP), :]
            s = jax.lax.dot_general(q_v[...], ck, NT, preferred_element_type=F32)
            m_new = jnp.maximum(m_prev, jnp.max(s, axis=1, keepdims=True))
            alpha = jnp.exp2(m_prev - m_new)
            p = jnp.exp2(s - m_new)
            l_new = l_prev * alpha + jnp.sum(p, axis=1, keepdims=True)
            acc = acc * alpha + jnp.dot(p.astype(BF16), ck, preferred_element_type=F32)
            return m_new, l_new, acc

        m0 = jnp.full((H, 1), -1e30, F32)
        l0 = jnp.zeros((H, 1), F32)
        a0 = jnp.zeros((H, Dc), F32)
        _, l_fin, acc = jax.lax.fori_loop(0, Sk // KV_STEP, kv_body, (m0, l0, a0))
        o_lat = acc / l_fin

        for b in range(NB):
            a_v[b] = o_lat[:, b * 128:(b + 1) * 128].astype(BF16)
        wait(N_UV)
        ctx = head_proj(wuv_v)

        wait(N_UV + 1)

        def wo_body(b, att):
            lo = jnp.concatenate(
                [jnp.where(row_h == b * HPB + j, ctx, 0.0) for j in range(HPB)], axis=1
            ).astype(BF16)
            rows = pl.ds(pl.multiple_of(b * HPB * D, HPB * D), HPB * D)
            return att + jnp.dot(lo, wo_v[rows, :], preferred_element_type=F32)
        att = jax.lax.fori_loop(0, H // HPB, wo_body, jnp.zeros((H, M), F32))
        x1 = x + ga * jnp.sum(att, axis=0, keepdims=True)

        h2 = jnp.broadcast_to((_ln(x1) * (1.0 + cb) + sb), (8, M)).astype(BF16)

        def gu_body(w, _):
            @pl.when(w == 0)
            def _():
                wait(N_UV + 2)

            @pl.when(w == 1)
            def _():
                wait(N_UV + 3)

            gu_v[w] = jnp.dot(h2, wgu_v[w], preferred_element_type=F32)
            return 0
        jax.lax.fori_loop(0, 2, gu_body, 0)
        act = _gelu(gu_v[0]) * gu_v[1]
        for i in range(Df // WD_STEP):
            act_v[i] = act[:, i * WD_STEP:(i + 1) * WD_STEP].astype(BF16)

        def wd_body(i, ffn):
            for k, a in enumerate(WD_DMAS[:-1]):
                @pl.when(i == a // WD_STEP)
                def _():
                    wait(N_WD + k)

            rows = pl.ds(pl.multiple_of(i * WD_STEP, WD_STEP), WD_STEP)
            return ffn + jnp.dot(act_v[i], wd_v[rows, :], preferred_element_type=F32)
        ffn = jax.lax.fori_loop(0, Df // WD_STEP, wd_body, jnp.zeros((8, M), F32))
        o_ref[0] = (x1 + gb * ffn[0:1]).astype(o_ref.dtype)

    hbm = pl.BlockSpec(memory_space=pl.ANY)
    return pl.pallas_call(
        kernel,
        in_specs=[hbm] * 11,
        out_specs=pl.BlockSpec(memory_space=pltpu.VMEM),
        out_shape=jax.ShapeDtypeStruct((1, Sq, M), A_x.dtype),
        scratch_shapes=[
            pltpu.VMEM((1, Sq, M), BF16),
            pltpu.VMEM((1, M), BF16),
            pltpu.VMEM((M, 6 * M), BF16),
            pltpu.VMEM((M * H, D), BF16),
            pltpu.VMEM((Dc * H, D), BF16),
            pltpu.VMEM((Sk, Dc), BF16),
            pltpu.VMEM((Dc * H, D), BF16),
            pltpu.VMEM((H * D, M), BF16),
            pltpu.VMEM((2, M, Df), BF16),
            pltpu.VMEM((Df, M), BF16),
            pltpu.VMEM((128, RB), BF16),
            pltpu.VMEM((NB, H, 128), BF16),
            pltpu.VMEM((H, Dc), BF16),
            pltpu.VMEM((2, 8, Df), F32),
            pltpu.VMEM((Df // WD_STEP, 8, WD_STEP), BF16),
            pltpu.SemaphoreType.DMA((WIN,)),
        ],
        compiler_params=pltpu.CompilerParams(vmem_limit_bytes=100 * 1024 * 1024),
    )(
        A_x, A_c_kv.reshape(Sk, Dc), A_w_q.reshape(M * H, D), A_w_uk.reshape(Dc * H, D),
        A_w_uv.reshape(Dc * H, D), A_w_o.reshape(H * D, M), B_w_gate, B_w_up, B_w_down,
        c, w_mod,
    )
```

```python
import math

import jax
import jax.numpy as jnp
import jax.experimental.pallas as pl
import jax.experimental.pallas.tpu as pltpu


F32 = jnp.float32
BF16 = jnp.bfloat16
EPS = 1e-5
NT = (((1,), (1,)), ((), ()))

KV_DMA = 4096
KV_STEP = 1024
WD_STEP = 256
WD_DMAS = (0, 1024, 1536, 1664, 1792)
WD_MXU_DMAS = 2
WIN = 3


def _ln(x):
    m = jnp.mean(x, axis=-1, keepdims=True)
    d = x - m
    v = jnp.mean(d * d, axis=-1, keepdims=True)
    return d * jax.lax.rsqrt(v + EPS)


def _gelu(x):
    k = math.sqrt(2.0 / math.pi)
    return 0.5 * x * (1.0 + jnp.tanh(k * (x + 0.044715 * (x * x * x))))


@jax.jit
def pallas_adaLN_cond__compressed_kv_cla__glu_gated_geglu__decode_kernel(
    A_x: jax.Array,
    A_c_kv: jax.Array,
    A_w_q: jax.Array,
    A_w_uk: jax.Array,
    A_w_uv: jax.Array,
    A_w_o: jax.Array,
    B_x: jax.Array,
    B_w_gate: jax.Array,
    B_w_up: jax.Array,
    B_w_down: jax.Array,
    c: jax.Array,
    w_mod: jax.Array,
):
    del B_x
    _, Sq, M = A_x.shape
    _, Sk, Dc = A_c_kv.shape
    _, H, D = A_w_q.shape
    Df = B_w_gate.shape[1]
    assert (Sq, H, D) == (1, 32, 128) and M == Dc and M % 128 == 0
    assert Sk % KV_DMA == 0 and KV_DMA % KV_STEP == 0
    assert Df == WD_DMAS[-1] and all(b % WD_STEP == 0 for b in WD_DMAS[:WD_MXU_DMAS + 1])
    NKV = Sk // KV_DMA
    NB = M // 128
    RB = 128 * H
    HPB = 8
    scale = float(D) ** -0.5 * math.log2(math.e)

    def kernel(x_hbm, ckv_hbm, wq_hbm, wuk_hbm, wuv_hbm, wo_hbm, wg_hbm, wu_hbm, wd_hbm,
               c_hbm, wmod_hbm, o_ref,
               x_v, c_v, wmod_v, wq_v, wuk_v, ckv_v, wuv_v, wo_v, wgu_v, wd_v,
               e_v, a_v, q_v, gu_v, act_v, acol_v, sem):
        pairs = [(wmod_hbm, wmod_v), (wq_hbm, wq_v), (wuk_hbm, wuk_v)]
        N_KV0 = len(pairs)
        pairs += [(ckv_hbm.at[pl.ds(i * KV_DMA, KV_DMA)], ckv_v.at[pl.ds(i * KV_DMA, KV_DMA)])
                  for i in range(NKV)]
        N_UV = len(pairs)
        pairs += [(wuv_hbm, wuv_v), (wo_hbm, wo_v), (wg_hbm, wgu_v.at[0]), (wu_hbm, wgu_v.at[1])]
        N_WD = len(pairs)
        pairs += [(wd_hbm.at[pl.ds(a, b - a)], wd_v.at[pl.ds(a, b - a)])
                  for a, b in zip(WD_DMAS[:-1], WD_DMAS[1:])]

        def copy(n):
            return pltpu.make_async_copy(pairs[n][0], pairs[n][1], sem.at[n % WIN])

        def start(n):
            if n < len(pairs):
                copy(n).start()

        def wait(n):
            copy(n).wait()
            start(n + WIN)

        def kv_copy(i):
            rows = pl.ds(pl.multiple_of(i * KV_DMA, KV_DMA), KV_DMA)
            return pltpu.make_async_copy(ckv_hbm.at[rows], ckv_v.at[rows],
                                         sem.at[(N_KV0 + i) % WIN])

        cp_c = pltpu.make_async_copy(c_hbm, c_v, sem.at[0])
        cp_x = pltpu.make_async_copy(x_hbm, x_v, sem.at[0])
        start(0)
        cp_c.start()
        cp_x.start()
        for n in range(1, WIN):
            start(n)

        r_i = jax.lax.broadcasted_iota(jnp.int32, (128, RB), 0)
        n_i = jax.lax.broadcasted_iota(jnp.int32, (128, RB), 1)
        e_v[...] = jnp.where(r_i == n_i // H, 1.0, 0.0).astype(BF16)

        row_h = jax.lax.broadcasted_iota(jnp.int32, (H, 128), 0)
        diag = row_h == (jax.lax.broadcasted_iota(jnp.int32, (H, 128), 1) % H)

        def keep_diag(r):
            return jnp.concatenate(
                [jnp.where(diag, r[:, t * 128:(t + 1) * 128], 0.0) for t in range(RB // 128)],
                axis=1).astype(BF16)

        def head_proj(w_v):
            def body(b, out):
                rep = jnp.dot(a_v[b], e_v[...], preferred_element_type=F32)
                rows = pl.ds(pl.multiple_of(b * RB, RB), RB)
                return out + jnp.dot(keep_diag(rep), w_v[rows, :], preferred_element_type=F32)
            return jax.lax.fori_loop(0, NB, body, jnp.zeros((H, D), F32))

        copy(0).wait()
        cp_c.wait()
        cp_x.wait()
        start(WIN)
        cf = c_v[...].astype(F32)
        sc = (cf * jax.nn.sigmoid(cf)).astype(BF16)
        mod = jnp.dot(sc, wmod_v[...], preferred_element_type=F32)
        sa, ca, ga, sb, cb, gb = [mod[:, i * M:(i + 1) * M] for i in range(6)]
        x = x_v[0].astype(F32)
        h = _ln(x) * (1.0 + ca) + sa

        for b in range(NB):
            a_v[b] = jnp.broadcast_to(h[:, b * 128:(b + 1) * 128], (H, 128)).astype(BF16)
        wait(1)
        qb = head_proj(wq_v).astype(BF16)

        wait(2)

        def uk_body(b, _):
            rows = pl.ds(pl.multiple_of(b * RB, RB), RB)
            r = jax.lax.dot_general(qb, wuk_v[rows, :], NT, preferred_element_type=F32)
            qa = jax.lax.dot_general(keep_diag(r * scale), e_v[...], NT,
                                     preferred_element_type=F32)
            a_v[b] = qa.astype(BF16)
            return 0
        jax.lax.fori_loop(0, NB, uk_body, 0)
        q_v[...] = jnp.concatenate([a_v[b] for b in range(NB)], axis=1)

        SPD = KV_DMA // KV_STEP

        def kv_body(j, carry):
            m_prev, l_prev, acc = carry

            @pl.when(j % SPD == 0)
            def _():
                i = j // SPD
                kv_copy(i).wait()

                @pl.when(i + WIN < NKV)
                def _():
                    kv_copy(i + WIN).start()

                for t in range(WIN):
                    @pl.when(i + WIN == NKV + t)
                    def _():
                        start(N_UV + t)

            ck = ckv_v[pl.ds(pl.multiple_of(j * KV_STEP, KV_STEP), KV_STEP), :]
            s = jax.lax.dot_general(q_v[...], ck, NT, preferred_element_type=F32)
            m_new = jnp.maximum(m_prev, jnp.max(s, axis=1, keepdims=True))
            alpha = jnp.exp2(m_prev - m_new)
            p = jnp.exp2(s - m_new)
            l_new = l_prev * alpha + jnp.sum(p, axis=1, keepdims=True)
            acc = acc * alpha + jnp.dot(p.astype(BF16), ck, preferred_element_type=F32)
            return m_new, l_new, acc

        m0 = jnp.full((H, 1), -1e30, F32)
        l0 = jnp.zeros((H, 1), F32)
        a0 = jnp.zeros((H, Dc), F32)
        _, l_fin, acc = jax.lax.fori_loop(0, Sk // KV_STEP, kv_body, (m0, l0, a0))
        o_lat = acc / l_fin

        for b in range(NB):
            a_v[b] = o_lat[:, b * 128:(b + 1) * 128].astype(BF16)
        wait(N_UV)
        ctx = head_proj(wuv_v)

        wait(N_UV + 1)

        def wo_body(b, att):
            lo = jnp.concatenate(
                [jnp.where(row_h == b * HPB + j, ctx, 0.0) for j in range(HPB)], axis=1
            ).astype(BF16)
            rows = pl.ds(pl.multiple_of(b * HPB * D, HPB * D), HPB * D)
            return att + jnp.dot(lo, wo_v[rows, :], preferred_element_type=F32)
        att = jax.lax.fori_loop(0, H // HPB, wo_body, jnp.zeros((H, M), F32))
        x1 = x + ga * jnp.sum(att, axis=0, keepdims=True)

        h2 = jnp.broadcast_to((_ln(x1) * (1.0 + cb) + sb), (8, M)).astype(BF16)

        def gu_body(w, _):
            @pl.when(w == 0)
            def _():
                wait(N_UV + 2)

            @pl.when(w == 1)
            def _():
                wait(N_UV + 3)

            gu_v[w] = jnp.dot(h2, wgu_v[w], preferred_element_type=F32)
            return 0
        jax.lax.fori_loop(0, 2, gu_body, 0)
        act = _gelu(gu_v[0]) * gu_v[1]
        for i in range(Df // WD_STEP):
            act_v[i] = act[:, i * WD_STEP:(i + 1) * WD_STEP].astype(BF16)

        NV = len(WD_DMAS) - 1 - WD_MXU_DMAS
        F0 = WD_DMAS[WD_MXU_DMAS]
        LAST = (Df - F0) // NV
        for k in range(NV):
            a_k = act[0:1, F0 + k * LAST:F0 + (k + 1) * LAST].astype(BF16).astype(F32)
            acol_v[k] = jnp.broadcast_to(a_k, (128, LAST)).T

        def wd_body(i, ffn):
            for k, a in enumerate(WD_DMAS[:WD_MXU_DMAS]):
                @pl.when(i == a // WD_STEP)
                def _():
                    wait(N_WD + k)

            rows = pl.ds(pl.multiple_of(i * WD_STEP, WD_STEP), WD_STEP)
            return ffn + jnp.dot(act_v[i], wd_v[rows, :], preferred_element_type=F32)
        ffn = jax.lax.fori_loop(0, F0 // WD_STEP, wd_body, jnp.zeros((8, M), F32))
        base = x1 + gb * ffn[0:1]

        def vpu_body(k, part):
            for kk in range(NV):
                @pl.when(k == kk)
                def _():
                    wait(N_WD + WD_MXU_DMAS + kk)

            w_k = wd_v[pl.ds(pl.multiple_of(F0 + k * LAST, LAST), LAST), :].astype(F32)
            a_c = acol_v[k]
            prod = jnp.concatenate([w_k[:, t * 128:(t + 1) * 128] * a_c for t in range(M // 128)], axis=1)
            return part + jnp.sum(prod.reshape(LAST // 8, 8, M), axis=0)
        part = jax.lax.fori_loop(0, NV, vpu_body, jnp.zeros((8, M), F32))
        o_ref[0] = (base + gb * jnp.sum(part, axis=0, keepdims=True)).astype(o_ref.dtype)

    hbm = pl.BlockSpec(memory_space=pl.ANY)
    return pl.pallas_call(
        kernel,
        in_specs=[hbm] * 11,
        out_specs=pl.BlockSpec(memory_space=pltpu.VMEM),
        out_shape=jax.ShapeDtypeStruct((1, Sq, M), A_x.dtype),
        scratch_shapes=[
            pltpu.VMEM((1, Sq, M), BF16),
            pltpu.VMEM((1, M), BF16),
            pltpu.VMEM((M, 6 * M), BF16),
            pltpu.VMEM((M * H, D), BF16),
            pltpu.VMEM((Dc * H, D), BF16),
            pltpu.VMEM((Sk, Dc), BF16),
            pltpu.VMEM((Dc * H, D), BF16),
            pltpu.VMEM((H * D, M), BF16),
            pltpu.VMEM((2, M, Df), BF16),
            pltpu.VMEM((Df, M), BF16),
            pltpu.VMEM((128, RB), BF16),
            pltpu.VMEM((NB, H, 128), BF16),
            pltpu.VMEM((H, Dc), BF16),
            pltpu.VMEM((2, 8, Df), F32),
            pltpu.VMEM((Df // WD_STEP, 8, WD_STEP), BF16),
            pltpu.VMEM((len(WD_DMAS) - 1 - WD_MXU_DMAS, (Df - WD_DMAS[WD_MXU_DMAS]) // (len(WD_DMAS) - 1 - WD_MXU_DMAS), 128), F32),
            pltpu.SemaphoreType.DMA((WIN,)),
        ],
        compiler_params=pltpu.CompilerParams(vmem_limit_bytes=100 * 1024 * 1024),
    )(
        A_x, A_c_kv.reshape(Sk, Dc), A_w_q.reshape(M * H, D), A_w_uk.reshape(Dc * H, D),
        A_w_uv.reshape(Dc * H, D), A_w_o.reshape(H * D, M), B_w_gate, B_w_up, B_w_down,
        c, w_mod,
    )
```

```python
import math

import jax
import jax.numpy as jnp
import jax.experimental.pallas as pl
import jax.experimental.pallas.tpu as pltpu


F32 = jnp.float32
BF16 = jnp.bfloat16
EPS = 1e-5
NT = (((1,), (1,)), ((), ()))

KV_DMA = 4096
KV_STEP = 1024
WD_STEP = 256
WD_DMAS = (0, 1024, 1536, 1728, 1792)
WD_MXU_DMAS = 2
VPU_STEP = 64
WIN = 3


def _ln(x):
    m = jnp.mean(x, axis=-1, keepdims=True)
    d = x - m
    v = jnp.mean(d * d, axis=-1, keepdims=True)
    return d * jax.lax.rsqrt(v + EPS)


def _gelu(x):
    k = math.sqrt(2.0 / math.pi)
    return 0.5 * x * (1.0 + jnp.tanh(k * (x + 0.044715 * (x * x * x))))


@jax.jit
def pallas_adaLN_cond__compressed_kv_cla__glu_gated_geglu__decode_kernel(
    A_x: jax.Array,
    A_c_kv: jax.Array,
    A_w_q: jax.Array,
    A_w_uk: jax.Array,
    A_w_uv: jax.Array,
    A_w_o: jax.Array,
    B_x: jax.Array,
    B_w_gate: jax.Array,
    B_w_up: jax.Array,
    B_w_down: jax.Array,
    c: jax.Array,
    w_mod: jax.Array,
):
    del B_x
    _, Sq, M = A_x.shape
    _, Sk, Dc = A_c_kv.shape
    _, H, D = A_w_q.shape
    Df = B_w_gate.shape[1]
    assert (Sq, H, D) == (1, 32, 128) and M == Dc and M % 128 == 0
    assert Sk % KV_DMA == 0 and KV_DMA % KV_STEP == 0
    assert Df == WD_DMAS[-1] and all(b % WD_STEP == 0 for b in WD_DMAS[:WD_MXU_DMAS + 1])
    NKV = Sk // KV_DMA
    NB = M // 128
    RB = 128 * H
    HPB = 8
    F0 = WD_DMAS[WD_MXU_DMAS]
    scale = float(D) ** -0.5 * math.log2(math.e)

    def kernel(x_hbm, ckv_hbm, wq_hbm, wuk_hbm, wuv_hbm, wo_hbm, wg_hbm, wu_hbm, wd_hbm,
               c_hbm, wmod_hbm, o_ref,
               x_v, c_v, wmod_v, wq_v, wuk_v, ckv_v, wuv_v, wo_v, wgu_v, wd_v,
               e_v, a_v, q_v, gu_v, act_v, acol_v, sem):
        pairs = [(wmod_hbm, wmod_v), (wq_hbm, wq_v), (wuk_hbm, wuk_v)]
        N_KV0 = len(pairs)
        pairs += [(ckv_hbm.at[pl.ds(i * KV_DMA, KV_DMA)], ckv_v.at[pl.ds(i * KV_DMA, KV_DMA)])
                  for i in range(NKV)]
        N_UV = len(pairs)
        pairs += [(wuv_hbm, wuv_v), (wo_hbm, wo_v), (wg_hbm, wgu_v.at[0]), (wu_hbm, wgu_v.at[1])]
        N_WD = len(pairs)
        pairs += [(wd_hbm.at[pl.ds(a, b - a)], wd_v.at[pl.ds(a, b - a)])
                  for a, b in zip(WD_DMAS[:-1], WD_DMAS[1:])]

        def copy(n):
            return pltpu.make_async_copy(pairs[n][0], pairs[n][1], sem.at[n % WIN])

        def start(n):
            if n < len(pairs):
                copy(n).start()

        def wait(n):
            copy(n).wait()
            start(n + WIN)

        def kv_copy(i):
            rows = pl.ds(pl.multiple_of(i * KV_DMA, KV_DMA), KV_DMA)
            return pltpu.make_async_copy(ckv_hbm.at[rows], ckv_v.at[rows],
                                         sem.at[(N_KV0 + i) % WIN])

        cp_c = pltpu.make_async_copy(c_hbm, c_v, sem.at[0])
        cp_x = pltpu.make_async_copy(x_hbm, x_v, sem.at[0])
        start(0)
        cp_c.start()
        cp_x.start()
        for n in range(1, WIN):
            start(n)

        r_i = jax.lax.broadcasted_iota(jnp.int32, (128, RB), 0)
        n_i = jax.lax.broadcasted_iota(jnp.int32, (128, RB), 1)
        e_v[...] = jnp.where(r_i == n_i // H, 1.0, 0.0).astype(BF16)

        row_h = jax.lax.broadcasted_iota(jnp.int32, (H, 128), 0)
        diag = row_h == (jax.lax.broadcasted_iota(jnp.int32, (H, 128), 1) % H)

        def keep_diag(r):
            return jnp.concatenate(
                [jnp.where(diag, r[:, t * 128:(t + 1) * 128], 0.0) for t in range(RB // 128)],
                axis=1).astype(BF16)

        def head_proj(w_v):
            def body(b, out):
                rep = jnp.dot(a_v[b], e_v[...], preferred_element_type=F32)
                rows = pl.ds(pl.multiple_of(b * RB, RB), RB)
                return out + jnp.dot(keep_diag(rep), w_v[rows, :], preferred_element_type=F32)
            return jax.lax.fori_loop(0, NB, body, jnp.zeros((H, D), F32))

        copy(0).wait()
        cp_c.wait()
        cp_x.wait()
        start(WIN)
        cf = c_v[...].astype(F32)
        sc = (cf * jax.nn.sigmoid(cf)).astype(BF16)
        mod = jnp.dot(sc, wmod_v[...], preferred_element_type=F32)
        sa, ca, ga, sb, cb, gb = [mod[:, i * M:(i + 1) * M] for i in range(6)]
        x = x_v[0].astype(F32)
        h = _ln(x) * (1.0 + ca) + sa

        for b in range(NB):
            a_v[b] = jnp.broadcast_to(h[:, b * 128:(b + 1) * 128], (H, 128)).astype(BF16)
        wait(1)
        qb = head_proj(wq_v).astype(BF16)

        wait(2)

        def uk_body(b, _):
            rows = pl.ds(pl.multiple_of(b * RB, RB), RB)
            r = jax.lax.dot_general(qb, wuk_v[rows, :], NT, preferred_element_type=F32)
            qa = jax.lax.dot_general(keep_diag(r * scale), e_v[...], NT,
                                     preferred_element_type=F32)
            a_v[b] = qa.astype(BF16)
            return 0
        jax.lax.fori_loop(0, NB, uk_body, 0)
        q_v[...] = jnp.concatenate([a_v[b] for b in range(NB)], axis=1)

        SPD = KV_DMA // KV_STEP

        def kv_body(j, carry):
            m_prev, l_prev, acc = carry

            @pl.when(j % SPD == 0)
            def _():
                i = j // SPD
                kv_copy(i).wait()

                @pl.when(i + WIN < NKV)
                def _():
                    kv_copy(i + WIN).start()

                for t in range(WIN):
                    @pl.when(i + WIN == NKV + t)
                    def _():
                        start(N_UV + t)

            ck = ckv_v[pl.ds(pl.multiple_of(j * KV_STEP, KV_STEP), KV_STEP), :]
            s = jax.lax.dot_general(q_v[...], ck, NT, preferred_element_type=F32)
            m_new = jnp.maximum(m_prev, jnp.max(s, axis=1, keepdims=True))
            alpha = jnp.exp2(m_prev - m_new)
            p = jnp.exp2(s - m_new)
            l_new = l_prev * alpha + jnp.sum(p, axis=1, keepdims=True)
            acc = acc * alpha + jnp.dot(p.astype(BF16), ck, preferred_element_type=F32)
            return m_new, l_new, acc

        m0 = jnp.full((H, 1), -jnp.inf, F32)
        l0 = jnp.zeros((H, 1), F32)
        a0 = jnp.zeros((H, Dc), F32)
        _, l_fin, acc = jax.lax.fori_loop(0, Sk // KV_STEP, kv_body, (m0, l0, a0))
        o_lat = acc / l_fin

        for b in range(NB):
            a_v[b] = o_lat[:, b * 128:(b + 1) * 128].astype(BF16)
        wait(N_UV)
        ctx = head_proj(wuv_v)

        wait(N_UV + 1)

        def wo_body(b, att):
            lo = jnp.concatenate(
                [jnp.where(row_h == b * HPB + j, ctx, 0.0) for j in range(HPB)], axis=1
            ).astype(BF16)
            rows = pl.ds(pl.multiple_of(b * HPB * D, HPB * D), HPB * D)
            return att + jnp.dot(lo, wo_v[rows, :], preferred_element_type=F32)
        att = jax.lax.fori_loop(0, H // HPB, wo_body, jnp.zeros((H, M), F32))
        x1 = x + ga * jnp.sum(att, axis=0, keepdims=True)

        h2 = jnp.broadcast_to((_ln(x1) * (1.0 + cb) + sb), (8, M)).astype(BF16)

        def gu_body(w, _):
            @pl.when(w == 0)
            def _():
                wait(N_UV + 2)

            @pl.when(w == 1)
            def _():
                wait(N_UV + 3)

            gu_v[w] = jnp.dot(h2, wgu_v[w], preferred_element_type=F32)
            return 0
        jax.lax.fori_loop(0, 2, gu_body, 0)
        act = _gelu(gu_v[0]) * gu_v[1]
        for i in range(F0 // WD_STEP):
            act_v[i] = act[:, i * WD_STEP:(i + 1) * WD_STEP].astype(BF16)

        for k in range((Df - F0) // VPU_STEP):
            a_k = act[0:1, F0 + k * VPU_STEP:F0 + (k + 1) * VPU_STEP].astype(BF16).astype(F32)
            acol_v[k] = jnp.broadcast_to(a_k, (128, VPU_STEP)).T

        def wd_body(i, ffn):
            for k, a in enumerate(WD_DMAS[:WD_MXU_DMAS]):
                @pl.when(i == a // WD_STEP)
                def _():
                    wait(N_WD + k)

            rows = pl.ds(pl.multiple_of(i * WD_STEP, WD_STEP), WD_STEP)
            return ffn + jnp.dot(act_v[i], wd_v[rows, :], preferred_element_type=F32)
        ffn = jax.lax.fori_loop(0, F0 // WD_STEP, wd_body, jnp.zeros((8, M), F32))
        base = x1 + gb * ffn[0:1]

        def vpu_body(i, part):
            for k in range(WD_MXU_DMAS, len(WD_DMAS) - 1):
                @pl.when(i == (WD_DMAS[k] - F0) // VPU_STEP)
                def _():
                    wait(N_WD + k)

            rows = pl.ds(pl.multiple_of(F0 + i * VPU_STEP, VPU_STEP), VPU_STEP)
            w_i = wd_v[rows, :].astype(F32)
            a_c = acol_v[i]
            prod = jnp.concatenate(
                [w_i[:, t * 128:(t + 1) * 128] * a_c for t in range(M // 128)], axis=1)
            return part + jnp.sum(prod.reshape(VPU_STEP // 8, 8, M), axis=0)
        part = jax.lax.fori_loop(0, (Df - F0) // VPU_STEP, vpu_body, jnp.zeros((8, M), F32))
        o_ref[0] = (base + gb * jnp.sum(part, axis=0, keepdims=True)).astype(o_ref.dtype)

    hbm = pl.BlockSpec(memory_space=pl.ANY)
    return pl.pallas_call(
        kernel,
        in_specs=[hbm] * 11,
        out_specs=pl.BlockSpec(memory_space=pltpu.VMEM),
        out_shape=jax.ShapeDtypeStruct((1, Sq, M), A_x.dtype),
        scratch_shapes=[
            pltpu.VMEM((1, Sq, M), BF16),
            pltpu.VMEM((1, M), BF16),
            pltpu.VMEM((M, 6 * M), BF16),
            pltpu.VMEM((M * H, D), BF16),
            pltpu.VMEM((Dc * H, D), BF16),
            pltpu.VMEM((Sk, Dc), BF16),
            pltpu.VMEM((Dc * H, D), BF16),
            pltpu.VMEM((H * D, M), BF16),
            pltpu.VMEM((2, M, Df), BF16),
            pltpu.VMEM((Df, M), BF16),
            pltpu.VMEM((128, RB), BF16),
            pltpu.VMEM((NB, H, 128), BF16),
            pltpu.VMEM((H, Dc), BF16),
            pltpu.VMEM((2, 8, Df), F32),
            pltpu.VMEM((F0 // WD_STEP, 8, WD_STEP), BF16),
            pltpu.VMEM(((Df - F0) // VPU_STEP, VPU_STEP, 128), F32),
            pltpu.SemaphoreType.DMA((WIN,)),
        ],
        compiler_params=pltpu.CompilerParams(vmem_limit_bytes=100 * 1024 * 1024),
    )(
        A_x, A_c_kv.reshape(Sk, Dc), A_w_q.reshape(M * H, D), A_w_uk.reshape(Dc * H, D),
        A_w_uv.reshape(Dc * H, D), A_w_o.reshape(H * D, M), B_w_gate, B_w_up, B_w_down,
        c, w_mod,
    )
```

```python
import math

import jax
import jax.numpy as jnp
import jax.experimental.pallas as pl
import jax.experimental.pallas.tpu as pltpu


F32 = jnp.float32
BF16 = jnp.bfloat16
EPS = 1e-5
NT = (((1,), (1,)), ((), ()))

KV_DMA = 4096
KV_STEP = 1024
WD_STEP = 256
WD_DMAS = (0, 768, 1280, 1408, 1536, 1664, 1728, 1792)
WD_MXU_DMAS = 2
VPU_STEP = 64
WIN = 8


def _ln(x):
    m = jnp.mean(x, axis=-1, keepdims=True)
    d = x - m
    v = jnp.mean(d * d, axis=-1, keepdims=True)
    return d * jax.lax.rsqrt(v + EPS)


def _gelu(x):
    k = math.sqrt(2.0 / math.pi)
    return 0.5 * x * (1.0 + jnp.tanh(k * (x + 0.044715 * (x * x * x))))


@jax.jit
def pallas_adaLN_cond__compressed_kv_cla__glu_gated_geglu__decode_kernel(
    A_x: jax.Array,
    A_c_kv: jax.Array,
    A_w_q: jax.Array,
    A_w_uk: jax.Array,
    A_w_uv: jax.Array,
    A_w_o: jax.Array,
    B_x: jax.Array,
    B_w_gate: jax.Array,
    B_w_up: jax.Array,
    B_w_down: jax.Array,
    c: jax.Array,
    w_mod: jax.Array,
):
    del B_x
    _, Sq, M = A_x.shape
    _, Sk, Dc = A_c_kv.shape
    _, H, D = A_w_q.shape
    Df = B_w_gate.shape[1]
    assert (Sq, H, D) == (1, 32, 128) and M == Dc and M % 128 == 0
    assert Sk % KV_DMA == 0 and KV_DMA % KV_STEP == 0
    assert Df == WD_DMAS[-1] and all(b % WD_STEP == 0 for b in WD_DMAS[:WD_MXU_DMAS + 1])
    NKV = Sk // KV_DMA
    NB = M // 128
    RB = 128 * H
    HPB = 8
    F0 = WD_DMAS[WD_MXU_DMAS]
    scale = float(D) ** -0.5 * math.log2(math.e)

    def kernel(x_hbm, ckv_hbm, wq_hbm, wuk_hbm, wuv_hbm, wo_hbm, wg_hbm, wu_hbm, wd_hbm,
               c_hbm, wmod_hbm, o_ref,
               x_v, c_v, wmod_v, wq_v, wuk_v, ckv_v, wuv_v, wo_v, wgu_v, wd_v,
               e_v, a_v, q_v, gu_v, act_v, acol_v):
        pl.run_scoped(lambda sem: body(x_hbm, ckv_hbm, wq_hbm, wuk_hbm, wuv_hbm, wo_hbm, wg_hbm, wu_hbm, wd_hbm,
               c_hbm, wmod_hbm, o_ref,
               x_v, c_v, wmod_v, wq_v, wuk_v, ckv_v, wuv_v, wo_v, wgu_v, wd_v,
               e_v, a_v, q_v, gu_v, act_v, acol_v, sem), pltpu.SemaphoreType.DMA((WIN,)))

    def body(x_hbm, ckv_hbm, wq_hbm, wuk_hbm, wuv_hbm, wo_hbm, wg_hbm, wu_hbm, wd_hbm,
               c_hbm, wmod_hbm, o_ref,
               x_v, c_v, wmod_v, wq_v, wuk_v, ckv_v, wuv_v, wo_v, wgu_v, wd_v,
               e_v, a_v, q_v, gu_v, act_v, acol_v, sem):
        pairs = [(wmod_hbm, wmod_v), (wq_hbm, wq_v), (wuk_hbm, wuk_v)]
        N_KV0 = len(pairs)
        pairs += [(ckv_hbm.at[pl.ds(i * KV_DMA, KV_DMA)], ckv_v.at[pl.ds(i * KV_DMA, KV_DMA)])
                  for i in range(NKV)]
        N_UV = len(pairs)
        pairs += [(wuv_hbm, wuv_v), (wo_hbm, wo_v), (wg_hbm, wgu_v.at[0]), (wu_hbm, wgu_v.at[1])]
        N_WD = len(pairs)
        pairs += [(wd_hbm.at[pl.ds(a, b - a)], wd_v.at[pl.ds(a, b - a)])
                  for a, b in zip(WD_DMAS[:-1], WD_DMAS[1:])]

        def copy(n):
            return pltpu.make_async_copy(pairs[n][0], pairs[n][1], sem.at[n % WIN])

        def start(n):
            if n < len(pairs):
                copy(n).start()

        def wait(n):
            copy(n).wait()
            start(n + WIN)

        def kv_copy(i):
            rows = pl.ds(pl.multiple_of(i * KV_DMA, KV_DMA), KV_DMA)
            return pltpu.make_async_copy(ckv_hbm.at[rows], ckv_v.at[rows],
                                         sem.at[(N_KV0 + i) % WIN])

        cp_c = pltpu.make_async_copy(c_hbm, c_v, sem.at[0])
        cp_x = pltpu.make_async_copy(x_hbm, x_v, sem.at[0])
        start(0)
        cp_c.start()
        cp_x.start()
        for n in range(1, WIN):
            start(n)

        r_i = jax.lax.broadcasted_iota(jnp.int32, (128, RB), 0)
        n_i = jax.lax.broadcasted_iota(jnp.int32, (128, RB), 1)
        e_v[...] = jnp.where(r_i == n_i // H, 1.0, 0.0).astype(BF16)

        row_h = jax.lax.broadcasted_iota(jnp.int32, (H, 128), 0)
        diag = row_h == (jax.lax.broadcasted_iota(jnp.int32, (H, 128), 1) % H)

        def keep_diag(r):
            return jnp.concatenate(
                [jnp.where(diag, r[:, t * 128:(t + 1) * 128], 0.0) for t in range(RB // 128)],
                axis=1).astype(BF16)

        def head_proj(w_v):
            def body(b, out):
                rep = jnp.dot(a_v[b], e_v[...], preferred_element_type=F32)
                rows = pl.ds(pl.multiple_of(b * RB, RB), RB)
                return out + jnp.dot(keep_diag(rep), w_v[rows, :], preferred_element_type=F32)
            return jax.lax.fori_loop(0, NB, body, jnp.zeros((H, D), F32))

        copy(0).wait()
        cp_c.wait()
        cp_x.wait()
        start(WIN)
        cf = c_v[...].astype(F32)
        sc = (cf * jax.nn.sigmoid(cf)).astype(BF16)
        mod = jnp.dot(sc, wmod_v[...], preferred_element_type=F32)
        sa, ca, ga, sb, cb, gb = [mod[:, i * M:(i + 1) * M] for i in range(6)]
        x = x_v[0].astype(F32)
        h = _ln(x) * (1.0 + ca) + sa

        for b in range(NB):
            a_v[b] = jnp.broadcast_to(h[:, b * 128:(b + 1) * 128], (H, 128)).astype(BF16)
        wait(1)
        qb = head_proj(wq_v).astype(BF16)

        wait(2)

        def uk_body(b, _):
            rows = pl.ds(pl.multiple_of(b * RB, RB), RB)
            r = jax.lax.dot_general(qb, wuk_v[rows, :], NT, preferred_element_type=F32)
            qa = jax.lax.dot_general(keep_diag(r * scale), e_v[...], NT,
                                     preferred_element_type=F32)
            a_v[b] = qa.astype(BF16)
            return 0
        jax.lax.fori_loop(0, NB, uk_body, 0)
        q_v[...] = jnp.concatenate([a_v[b] for b in range(NB)], axis=1)

        SPD = KV_DMA // KV_STEP

        def kv_body(j, carry):
            m_prev, l_prev, acc = carry

            @pl.when(j % SPD == 0)
            def _():
                i = j // SPD
                kv_copy(i).wait()

                @pl.when(i + WIN < NKV)
                def _():
                    kv_copy(i + WIN).start()

                for t in range(WIN):
                    @pl.when(i + WIN == NKV + t)
                    def _():
                        start(N_UV + t)

            ck = ckv_v[pl.ds(pl.multiple_of(j * KV_STEP, KV_STEP), KV_STEP), :]
            s = jax.lax.dot_general(q_v[...], ck, NT, preferred_element_type=F32)
            m_new = jnp.maximum(m_prev, jnp.max(s, axis=1, keepdims=True))
            alpha = jnp.exp2(m_prev - m_new)
            p = jnp.exp2(s - m_new)
            l_new = l_prev * alpha + jnp.sum(p, axis=1, keepdims=True)
            acc = acc * alpha + jnp.dot(p.astype(BF16), ck, preferred_element_type=F32)
            return m_new, l_new, acc

        m0 = jnp.full((H, 1), -jnp.inf, F32)
        l0 = jnp.zeros((H, 1), F32)
        a0 = jnp.zeros((H, Dc), F32)
        _, l_fin, acc = jax.lax.fori_loop(0, Sk // KV_STEP, kv_body, (m0, l0, a0))
        o_lat = acc / l_fin

        for b in range(NB):
            a_v[b] = o_lat[:, b * 128:(b + 1) * 128].astype(BF16)
        wait(N_UV)
        ctx = head_proj(wuv_v)

        wait(N_UV + 1)

        def wo_body(b, att):
            lo = jnp.concatenate(
                [jnp.where(row_h == b * HPB + j, ctx, 0.0) for j in range(HPB)], axis=1
            ).astype(BF16)
            rows = pl.ds(pl.multiple_of(b * HPB * D, HPB * D), HPB * D)
            return att + jnp.dot(lo, wo_v[rows, :], preferred_element_type=F32)
        att = jax.lax.fori_loop(0, H // HPB, wo_body, jnp.zeros((H, M), F32))
        x1 = x + ga * jnp.sum(att, axis=0, keepdims=True)

        h2 = jnp.broadcast_to((_ln(x1) * (1.0 + cb) + sb), (8, M)).astype(BF16)

        def gu_body(w, _):
            @pl.when(w == 0)
            def _():
                wait(N_UV + 2)

            @pl.when(w == 1)
            def _():
                wait(N_UV + 3)

            gu_v[w] = jnp.dot(h2, wgu_v[w], preferred_element_type=F32)
            return 0
        jax.lax.fori_loop(0, 2, gu_body, 0)
        act = _gelu(gu_v[0]) * gu_v[1]
        for i in range(F0 // WD_STEP):
            act_v[i] = act[:, i * WD_STEP:(i + 1) * WD_STEP].astype(BF16)

        for k in range((Df - F0) // VPU_STEP):
            a_k = act[0:1, F0 + k * VPU_STEP:F0 + (k + 1) * VPU_STEP].astype(BF16).astype(F32)
            acol_v[k] = jnp.broadcast_to(a_k, (128, VPU_STEP)).T

        def wd_body(i, ffn):
            for k, a in enumerate(WD_DMAS[:WD_MXU_DMAS]):
                @pl.when(i == a // WD_STEP)
                def _():
                    wait(N_WD + k)

            rows = pl.ds(pl.multiple_of(i * WD_STEP, WD_STEP), WD_STEP)
            return ffn + jnp.dot(act_v[i], wd_v[rows, :], preferred_element_type=F32)
        ffn = jax.lax.fori_loop(0, F0 // WD_STEP, wd_body, jnp.zeros((8, M), F32))
        base = x1 + gb * ffn[0:1]

        def vpu_body(i, part):
            for k in range(WD_MXU_DMAS, len(WD_DMAS) - 1):
                @pl.when(i == (WD_DMAS[k] - F0) // VPU_STEP)
                def _():
                    wait(N_WD + k)

            rows = pl.ds(pl.multiple_of(F0 + i * VPU_STEP, VPU_STEP), VPU_STEP)
            w_i = wd_v[rows, :].astype(F32)
            a_c = acol_v[i]
            prod = jnp.concatenate(
                [w_i[:, t * 128:(t + 1) * 128] * a_c for t in range(M // 128)], axis=1)
            return part + jnp.sum(prod.reshape(VPU_STEP // 8, 8, M), axis=0)
        part = jax.lax.fori_loop(0, (Df - F0) // VPU_STEP, vpu_body, jnp.zeros((8, M), F32))
        o_ref[0] = (base + gb * jnp.sum(part, axis=0, keepdims=True)).astype(o_ref.dtype)

    hbm = pl.BlockSpec(memory_space=pl.ANY)
    return pl.pallas_call(
        kernel,
        in_specs=[hbm] * 11,
        out_specs=pl.BlockSpec(memory_space=pltpu.VMEM),
        out_shape=jax.ShapeDtypeStruct((1, Sq, M), A_x.dtype),
        scratch_shapes=[
            pltpu.VMEM((1, Sq, M), BF16),
            pltpu.VMEM((1, M), BF16),
            pltpu.VMEM((M, 6 * M), BF16),
            pltpu.VMEM((M * H, D), BF16),
            pltpu.VMEM((Dc * H, D), BF16),
            pltpu.VMEM((Sk, Dc), BF16),
            pltpu.VMEM((Dc * H, D), BF16),
            pltpu.VMEM((H * D, M), BF16),
            pltpu.VMEM((2, M, Df), BF16),
            pltpu.VMEM((Df, M), BF16),
            pltpu.VMEM((128, RB), BF16),
            pltpu.VMEM((NB, H, 128), BF16),
            pltpu.VMEM((H, Dc), BF16),
            pltpu.VMEM((2, 8, Df), F32),
            pltpu.VMEM((F0 // WD_STEP, 8, WD_STEP), BF16),
            pltpu.VMEM(((Df - F0) // VPU_STEP, VPU_STEP, 128), F32),
        ],
        compiler_params=pltpu.CompilerParams(vmem_limit_bytes=100 * 1024 * 1024),
    )(
        A_x, A_c_kv.reshape(Sk, Dc), A_w_q.reshape(M * H, D), A_w_uk.reshape(Dc * H, D),
        A_w_uv.reshape(Dc * H, D), A_w_o.reshape(H * D, M), B_w_gate, B_w_up, B_w_down,
        c, w_mod,
    )
```

```python
import math

import jax
import jax.numpy as jnp
import jax.experimental.pallas as pl
import jax.experimental.pallas.tpu as pltpu


F32 = jnp.float32
BF16 = jnp.bfloat16
EPS = 1e-5
NT = (((1,), (1,)), ((), ()))

KV_DMA = 1024
KV_STEP = 1024
WD_STEP = 256
WD_DMAS = (0, 768, 1280, 1408, 1536, 1664, 1728, 1792)
WD_MXU_DMAS = 2
VPU_STEP = 64
SIDE_ROWS = 384
SIDE_PIECES = 4
SIDE_STEPS = (1, 7, 13, 19, 25)
WIN = 8


def _ln(x):
    m = jnp.mean(x, axis=-1, keepdims=True)
    d = x - m
    v = jnp.mean(d * d, axis=-1, keepdims=True)
    return d * jax.lax.rsqrt(v + EPS)


def _gelu(x):
    k = math.sqrt(2.0 / math.pi)
    return 0.5 * x * (1.0 + jnp.tanh(k * (x + 0.044715 * (x * x * x))))


@jax.jit
def pallas_adaLN_cond__compressed_kv_cla__glu_gated_geglu__decode_kernel(
    A_x: jax.Array,
    A_c_kv: jax.Array,
    A_w_q: jax.Array,
    A_w_uk: jax.Array,
    A_w_uv: jax.Array,
    A_w_o: jax.Array,
    B_x: jax.Array,
    B_w_gate: jax.Array,
    B_w_up: jax.Array,
    B_w_down: jax.Array,
    c: jax.Array,
    w_mod: jax.Array,
):
    del B_x
    _, Sq, M = A_x.shape
    _, Sk, Dc = A_c_kv.shape
    _, H, D = A_w_q.shape
    Df = B_w_gate.shape[1]
    assert (Sq, H, D) == (1, 32, 128) and M == Dc and M % 128 == 0
    assert Sk % KV_DMA == 0 and KV_DMA % KV_STEP == 0
    assert Df == WD_DMAS[-1] and all(b % WD_STEP == 0 for b in WD_DMAS[:WD_MXU_DMAS + 1])
    assert SIDE_PIECES % 2 == 0 and len(SIDE_STEPS) == 2 * SIDE_PIECES - 3
    NKV = Sk // KV_DMA
    NB = M // 128
    RB = 128 * H
    HPB = 8
    F0 = WD_DMAS[WD_MXU_DMAS]
    scale = float(D) ** -0.5 * math.log2(math.e)

    def kernel(x_hbm, ckv_hbm, wq_hbm, wuk_hbm, wuv_hbm, wo_hbm, wg_hbm, wu_hbm, wd_hbm,
               c_hbm, wmod_hbm, o_ref,
               x_v, c_v, wmod_v, wq_v, wuk_v, ckv_v, wuv_v, wo_v, wgu_v, wd_v,
               e_v, a_v, q_v, gu_v, act_v, acol_v, side_s):
        pl.run_scoped(lambda sem, ssem: body(x_hbm, ckv_hbm, wq_hbm, wuk_hbm, wuv_hbm, wo_hbm, wg_hbm, wu_hbm, wd_hbm,
               c_hbm, wmod_hbm, o_ref,
               x_v, c_v, wmod_v, wq_v, wuk_v, ckv_v, wuv_v, wo_v, wgu_v, wd_v,
               e_v, a_v, q_v, gu_v, act_v, acol_v, side_s, sem, ssem),
                      pltpu.SemaphoreType.DMA((WIN,)), pltpu.SemaphoreType.DMA((4,)))

    def body(x_hbm, ckv_hbm, wq_hbm, wuk_hbm, wuv_hbm, wo_hbm, wg_hbm, wu_hbm, wd_hbm,
               c_hbm, wmod_hbm, o_ref,
               x_v, c_v, wmod_v, wq_v, wuk_v, ckv_v, wuv_v, wo_v, wgu_v, wd_v,
               e_v, a_v, q_v, gu_v, act_v, acol_v, side_s, sem, ssem):
        pairs = [(wmod_hbm, wmod_v), (wq_hbm, wq_v), (wuk_hbm, wuk_v)]
        N_KV0 = len(pairs)
        pairs += [(ckv_hbm.at[pl.ds(i * KV_DMA, KV_DMA)], ckv_v.at[pl.ds(i * KV_DMA, KV_DMA)])
                  for i in range(NKV)]
        N_UV = len(pairs)
        wo_main = pl.ds(SIDE_PIECES * SIDE_ROWS, H * D - SIDE_PIECES * SIDE_ROWS)
        pairs += [(wuv_hbm, wuv_v), (wo_hbm.at[wo_main], wo_v.at[wo_main]), (wg_hbm, wgu_v.at[0]), (wu_hbm, wgu_v.at[1])]
        N_WD = len(pairs)
        pairs += [(wd_hbm.at[pl.ds(a, b - a)], wd_v.at[pl.ds(a, b - a)])
                  for a, b in zip(WD_DMAS[:-1], WD_DMAS[1:])]

        def copy(n):
            return pltpu.make_async_copy(pairs[n][0], pairs[n][1], sem.at[n % WIN])

        def start(n):
            if n < len(pairs):
                copy(n).start()

        def wait(n):
            copy(n).wait()
            start(n + WIN)

        def kv_copy(i):
            rows = pl.ds(pl.multiple_of(i * KV_DMA, KV_DMA), KV_DMA)
            return pltpu.make_async_copy(ckv_hbm.at[rows], ckv_v.at[rows],
                                         sem.at[(N_KV0 + i) % WIN])

        def side(e):
            k = (e // 4) * 2 + e % 2
            rows = pl.ds(k * SIDE_ROWS, SIDE_ROWS)
            if e % 4 < 2:
                return pltpu.make_async_copy(wo_hbm.at[rows], side_s.at[k % 2], ssem.at[e % 4])
            return pltpu.make_async_copy(side_s.at[k % 2], wo_v.at[rows], ssem.at[e % 4])

        def side_step(e):
            side(e - 2).wait()
            if e < 2 * SIDE_PIECES:
                side(e).start()

        cp_c = pltpu.make_async_copy(c_hbm, c_v, sem.at[0])
        cp_x = pltpu.make_async_copy(x_hbm, x_v, sem.at[0])
        start(0)
        cp_c.start()
        cp_x.start()
        for n in range(1, WIN):
            start(n)
        side(0).start()
        side(1).start()

        r_i = jax.lax.broadcasted_iota(jnp.int32, (128, RB), 0)
        n_i = jax.lax.broadcasted_iota(jnp.int32, (128, RB), 1)
        e_v[...] = jnp.where(r_i == n_i // H, 1.0, 0.0).astype(BF16)

        row_h = jax.lax.broadcasted_iota(jnp.int32, (H, 128), 0)
        diag = row_h == (jax.lax.broadcasted_iota(jnp.int32, (H, 128), 1) % H)

        def keep_diag(r):
            return jnp.concatenate(
                [jnp.where(diag, r[:, t * 128:(t + 1) * 128], 0.0) for t in range(RB // 128)],
                axis=1).astype(BF16)

        def head_proj(w_v):
            def body(b, out):
                rep = jnp.dot(a_v[b], e_v[...], preferred_element_type=F32)
                rows = pl.ds(pl.multiple_of(b * RB, RB), RB)
                return out + jnp.dot(keep_diag(rep), w_v[rows, :], preferred_element_type=F32)
            return jax.lax.fori_loop(0, NB, body, jnp.zeros((H, D), F32))

        copy(0).wait()
        cp_c.wait()
        cp_x.wait()
        start(WIN)
        cf = c_v[...].astype(F32)
        sc = (cf * jax.nn.sigmoid(cf)).astype(BF16)
        mod = jnp.dot(sc, wmod_v[...], preferred_element_type=F32)
        sa, ca, ga, sb, cb, gb = [mod[:, i * M:(i + 1) * M] for i in range(6)]
        x = x_v[0].astype(F32)
        h = _ln(x) * (1.0 + ca) + sa

        for b in range(NB):
            a_v[b] = jnp.broadcast_to(h[:, b * 128:(b + 1) * 128], (H, 128)).astype(BF16)
        wait(1)
        side_step(2)
        qb = head_proj(wq_v).astype(BF16)

        wait(2)

        def uk_body(b, _):
            rows = pl.ds(pl.multiple_of(b * RB, RB), RB)
            r = jax.lax.dot_general(qb, wuk_v[rows, :], NT, preferred_element_type=F32)
            qa = jax.lax.dot_general(keep_diag(r * scale), e_v[...], NT,
                                     preferred_element_type=F32)
            a_v[b] = qa.astype(BF16)
            return 0
        jax.lax.fori_loop(0, NB, uk_body, 0)
        q_v[...] = jnp.concatenate([a_v[b] for b in range(NB)], axis=1)

        SPD = KV_DMA // KV_STEP

        def kv_body(j, carry):
            m_prev, l_prev, acc = carry

            @pl.when(j % SPD == 0)
            def _():
                i = j // SPD
                kv_copy(i).wait()

                @pl.when(i + WIN < NKV)
                def _():
                    kv_copy(i + WIN).start()

                for t in range(WIN):
                    @pl.when(i + WIN == NKV + t)
                    def _():
                        start(N_UV + t)

            for e, js in enumerate(SIDE_STEPS):
                @pl.when(j == js)
                def _():
                    side_step(3 + e)

            ck = ckv_v[pl.ds(pl.multiple_of(j * KV_STEP, KV_STEP), KV_STEP), :]
            s = jax.lax.dot_general(q_v[...], ck, NT, preferred_element_type=F32)
            m_new = jnp.maximum(m_prev, jnp.max(s, axis=1, keepdims=True))
            alpha = jnp.exp2(m_prev - m_new)
            p = jnp.exp2(s - m_new)
            l_new = l_prev * alpha + jnp.sum(p, axis=1, keepdims=True)
            acc = acc * alpha + jnp.dot(p.astype(BF16), ck, preferred_element_type=F32)
            return m_new, l_new, acc

        m0 = jnp.full((H, 1), -jnp.inf, F32)
        l0 = jnp.zeros((H, 1), F32)
        a0 = jnp.zeros((H, Dc), F32)
        _, l_fin, acc = jax.lax.fori_loop(0, Sk // KV_STEP, kv_body, (m0, l0, a0))
        o_lat = acc / l_fin

        for b in range(NB):
            a_v[b] = o_lat[:, b * 128:(b + 1) * 128].astype(BF16)
        wait(N_UV)
        ctx = head_proj(wuv_v)

        wait(N_UV + 1)
        side_step(2 * SIDE_PIECES)
        side_step(2 * SIDE_PIECES + 1)

        def wo_body(b, att):
            lo = jnp.concatenate(
                [jnp.where(row_h == b * HPB + j, ctx, 0.0) for j in range(HPB)], axis=1
            ).astype(BF16)
            rows = pl.ds(pl.multiple_of(b * HPB * D, HPB * D), HPB * D)
            return att + jnp.dot(lo, wo_v[rows, :], preferred_element_type=F32)
        att = jax.lax.fori_loop(0, H // HPB, wo_body, jnp.zeros((H, M), F32))
        x1 = x + ga * jnp.sum(att, axis=0, keepdims=True)

        h2 = jnp.broadcast_to((_ln(x1) * (1.0 + cb) + sb), (8, M)).astype(BF16)

        def gu_body(w, _):
            @pl.when(w == 0)
            def _():
                wait(N_UV + 2)

            @pl.when(w == 1)
            def _():
                wait(N_UV + 3)

            gu_v[w] = jnp.dot(h2, wgu_v[w], preferred_element_type=F32)
            return 0
        jax.lax.fori_loop(0, 2, gu_body, 0)
        act = _gelu(gu_v[0]) * gu_v[1]
        for i in range(F0 // WD_STEP):
            act_v[i] = act[:, i * WD_STEP:(i + 1) * WD_STEP].astype(BF16)

        for k in range((Df - F0) // VPU_STEP):
            a_k = act[0:1, F0 + k * VPU_STEP:F0 + (k + 1) * VPU_STEP].astype(BF16).astype(F32)
            acol_v[k] = jnp.broadcast_to(a_k, (128, VPU_STEP)).T

        def wd_body(i, ffn):
            for k, a in enumerate(WD_DMAS[:WD_MXU_DMAS]):
                @pl.when(i == a // WD_STEP)
                def _():
                    wait(N_WD + k)

            rows = pl.ds(pl.multiple_of(i * WD_STEP, WD_STEP), WD_STEP)
            return ffn + jnp.dot(act_v[i], wd_v[rows, :], preferred_element_type=F32)
        ffn = jax.lax.fori_loop(0, F0 // WD_STEP, wd_body, jnp.zeros((8, M), F32))
        base = x1 + gb * ffn[0:1]

        def vpu_body(i, part):
            for k in range(WD_MXU_DMAS, len(WD_DMAS) - 1):
                @pl.when(i == (WD_DMAS[k] - F0) // VPU_STEP)
                def _():
                    wait(N_WD + k)

            rows = pl.ds(pl.multiple_of(F0 + i * VPU_STEP, VPU_STEP), VPU_STEP)
            w_i = wd_v[rows, :].astype(F32)
            a_c = acol_v[i]
            prod = jnp.concatenate(
                [w_i[:, t * 128:(t + 1) * 128] * a_c for t in range(M // 128)], axis=1)
            return part + jnp.sum(prod.reshape(VPU_STEP // 8, 8, M), axis=0)
        part = jax.lax.fori_loop(0, (Df - F0) // VPU_STEP, vpu_body, jnp.zeros((8, M), F32))
        o_ref[0] = (base + gb * jnp.sum(part, axis=0, keepdims=True)).astype(o_ref.dtype)

    hbm = pl.BlockSpec(memory_space=pl.ANY)
    return pl.pallas_call(
        kernel,
        in_specs=[hbm] * 11,
        out_specs=pl.BlockSpec(memory_space=pltpu.VMEM),
        out_shape=jax.ShapeDtypeStruct((1, Sq, M), A_x.dtype),
        scratch_shapes=[
            pltpu.VMEM((1, Sq, M), BF16),
            pltpu.VMEM((1, M), BF16),
            pltpu.VMEM((M, 6 * M), BF16),
            pltpu.VMEM((M * H, D), BF16),
            pltpu.VMEM((Dc * H, D), BF16),
            pltpu.VMEM((Sk, Dc), BF16),
            pltpu.VMEM((Dc * H, D), BF16),
            pltpu.VMEM((H * D, M), BF16),
            pltpu.VMEM((2, M, Df), BF16),
            pltpu.VMEM((Df, M), BF16),
            pltpu.VMEM((128, RB), BF16),
            pltpu.VMEM((NB, H, 128), BF16),
            pltpu.VMEM((H, Dc), BF16),
            pltpu.VMEM((2, 8, Df), F32),
            pltpu.VMEM((F0 // WD_STEP, 8, WD_STEP), BF16),
            pltpu.VMEM(((Df - F0) // VPU_STEP, VPU_STEP, 128), F32),
            pltpu.SMEM((2, SIDE_ROWS, M), BF16),
        ],
        compiler_params=pltpu.CompilerParams(vmem_limit_bytes=100 * 1024 * 1024),
    )(
        A_x, A_c_kv.reshape(Sk, Dc), A_w_q.reshape(M * H, D), A_w_uk.reshape(Dc * H, D),
        A_w_uv.reshape(Dc * H, D), A_w_o.reshape(H * D, M), B_w_gate, B_w_up, B_w_down,
        c, w_mod,
    )
```

```python
import math

import jax
import jax.numpy as jnp
import jax.experimental.pallas as pl
import jax.experimental.pallas.tpu as pltpu


F32 = jnp.float32
BF16 = jnp.bfloat16
EPS = 1e-5
NT = (((1,), (1,)), ((), ()))

KV_DMA = 1024
KV_STEP = 1024
WD_STEP = 256
WD_DMAS = (0, 768, 1280, 1408, 1536, 1664, 1728, 1792)
WD_MXU_DMAS = 2
VPU_STEP = 64
SIDE_ROWS = 288
SIDE_WO = 5
SIDE_WD = 1
SIDE_STEPS = (0, 2, 6, 11, 15, 19, 24, 28, 31)
WIN = 8


def _ln(x):
    m = jnp.mean(x, axis=-1, keepdims=True)
    d = x - m
    v = jnp.mean(d * d, axis=-1, keepdims=True)
    return d * jax.lax.rsqrt(v + EPS)


def _gelu(x):
    k = math.sqrt(2.0 / math.pi)
    return 0.5 * x * (1.0 + jnp.tanh(k * (x + 0.044715 * (x * x * x))))


@jax.jit
def pallas_adaLN_cond__compressed_kv_cla__glu_gated_geglu__decode_kernel(
    A_x: jax.Array,
    A_c_kv: jax.Array,
    A_w_q: jax.Array,
    A_w_uk: jax.Array,
    A_w_uv: jax.Array,
    A_w_o: jax.Array,
    B_x: jax.Array,
    B_w_gate: jax.Array,
    B_w_up: jax.Array,
    B_w_down: jax.Array,
    c: jax.Array,
    w_mod: jax.Array,
):
    del B_x
    _, Sq, M = A_x.shape
    _, Sk, Dc = A_c_kv.shape
    _, H, D = A_w_q.shape
    Df = B_w_gate.shape[1]
    assert (Sq, H, D) == (1, 32, 128) and M == Dc and M % 128 == 0
    assert Sk % KV_DMA == 0 and KV_DMA % KV_STEP == 0
    assert Df == WD_DMAS[-1] and all(b % WD_STEP == 0 for b in WD_DMAS[:WD_MXU_DMAS + 1])
    SIDE_PIECES = SIDE_WO + SIDE_WD
    assert SIDE_PIECES % 2 == 0 and len(SIDE_STEPS) == 2 * SIDE_PIECES - 3
    WD0 = SIDE_WD * SIDE_ROWS
    wd_dmas = (WD0,) + WD_DMAS[1:]
    assert WD0 < WD_DMAS[1]
    NKV = Sk // KV_DMA
    NB = M // 128
    RB = 128 * H
    HPB = 8
    F0 = WD_DMAS[WD_MXU_DMAS]
    scale = float(D) ** -0.5 * math.log2(math.e)

    def kernel(x_hbm, ckv_hbm, wq_hbm, wuk_hbm, wuv_hbm, wo_hbm, wg_hbm, wu_hbm, wd_hbm,
               c_hbm, wmod_hbm, o_ref,
               x_v, c_v, wmod_v, wq_v, wuk_v, ckv_v, wuv_v, wo_v, wgu_v, wd_v,
               e_v, a_v, q_v, gu_v, act_v, acol_v, side_s):
        pl.run_scoped(lambda sem, ssem: body(x_hbm, ckv_hbm, wq_hbm, wuk_hbm, wuv_hbm, wo_hbm, wg_hbm, wu_hbm, wd_hbm,
               c_hbm, wmod_hbm, o_ref,
               x_v, c_v, wmod_v, wq_v, wuk_v, ckv_v, wuv_v, wo_v, wgu_v, wd_v,
               e_v, a_v, q_v, gu_v, act_v, acol_v, side_s, sem, ssem),
                      pltpu.SemaphoreType.DMA((WIN,)), pltpu.SemaphoreType.DMA((4,)))

    def body(x_hbm, ckv_hbm, wq_hbm, wuk_hbm, wuv_hbm, wo_hbm, wg_hbm, wu_hbm, wd_hbm,
               c_hbm, wmod_hbm, o_ref,
               x_v, c_v, wmod_v, wq_v, wuk_v, ckv_v, wuv_v, wo_v, wgu_v, wd_v,
               e_v, a_v, q_v, gu_v, act_v, acol_v, side_s, sem, ssem):
        pairs = [(wmod_hbm, wmod_v), (wq_hbm, wq_v), (wuk_hbm, wuk_v)]
        N_KV0 = len(pairs)
        pairs += [(ckv_hbm.at[pl.ds(i * KV_DMA, KV_DMA)], ckv_v.at[pl.ds(i * KV_DMA, KV_DMA)])
                  for i in range(NKV)]
        N_UV = len(pairs)
        wo_main = pl.ds(SIDE_WO * SIDE_ROWS, H * D - SIDE_WO * SIDE_ROWS)
        pairs += [(wuv_hbm, wuv_v), (wo_hbm.at[wo_main], wo_v.at[wo_main]), (wg_hbm, wgu_v.at[0]), (wu_hbm, wgu_v.at[1])]
        N_WD = len(pairs)
        pairs += [(wd_hbm.at[pl.ds(a, b - a)], wd_v.at[pl.ds(a, b - a)])
                  for a, b in zip(wd_dmas[:-1], wd_dmas[1:])]

        def copy(n):
            return pltpu.make_async_copy(pairs[n][0], pairs[n][1], sem.at[n % WIN])

        def start(n):
            if n < len(pairs):
                copy(n).start()

        def wait(n):
            copy(n).wait()
            start(n + WIN)

        def kv_copy(i):
            rows = pl.ds(pl.multiple_of(i * KV_DMA, KV_DMA), KV_DMA)
            return pltpu.make_async_copy(ckv_hbm.at[rows], ckv_v.at[rows],
                                         sem.at[(N_KV0 + i) % WIN])

        def side(e):
            k = (e // 4) * 2 + e % 2
            src, dst, k0 = (wo_hbm, wo_v, 0) if k < SIDE_WO else (wd_hbm, wd_v, SIDE_WO)
            rows = pl.ds((k - k0) * SIDE_ROWS, SIDE_ROWS)
            if e % 4 < 2:
                return pltpu.make_async_copy(src.at[rows], side_s.at[k % 2], ssem.at[e % 4])
            return pltpu.make_async_copy(side_s.at[k % 2], dst.at[rows], ssem.at[e % 4])

        def side_step(e):
            side(e - 2).wait()
            if e < 2 * SIDE_PIECES:
                side(e).start()

        cp_c = pltpu.make_async_copy(c_hbm, c_v, sem.at[0])
        cp_x = pltpu.make_async_copy(x_hbm, x_v, sem.at[0])
        start(0)
        cp_c.start()
        cp_x.start()
        for n in range(1, WIN):
            start(n)
        side(0).start()
        side(1).start()

        r_i = jax.lax.broadcasted_iota(jnp.int32, (128, RB), 0)
        n_i = jax.lax.broadcasted_iota(jnp.int32, (128, RB), 1)
        e_v[...] = jnp.where(r_i == n_i // H, 1.0, 0.0).astype(BF16)

        row_h = jax.lax.broadcasted_iota(jnp.int32, (H, 128), 0)
        diag = row_h == (jax.lax.broadcasted_iota(jnp.int32, (H, 128), 1) % H)

        def keep_diag(r):
            return jnp.concatenate(
                [jnp.where(diag, r[:, t * 128:(t + 1) * 128], 0.0) for t in range(RB // 128)],
                axis=1).astype(BF16)

        def head_proj(w_v):
            def body(b, out):
                rep = jnp.dot(a_v[b], e_v[...], preferred_element_type=F32)
                rows = pl.ds(pl.multiple_of(b * RB, RB), RB)
                return out + jnp.dot(keep_diag(rep), w_v[rows, :], preferred_element_type=F32)
            return jax.lax.fori_loop(0, NB, body, jnp.zeros((H, D), F32))

        copy(0).wait()
        cp_c.wait()
        cp_x.wait()
        start(WIN)
        cf = c_v[...].astype(F32)
        sc = (cf * jax.nn.sigmoid(cf)).astype(BF16)
        mod = jnp.dot(sc, wmod_v[...], preferred_element_type=F32)
        sa, ca, ga, sb, cb, gb = [mod[:, i * M:(i + 1) * M] for i in range(6)]
        x = x_v[0].astype(F32)
        h = _ln(x) * (1.0 + ca) + sa

        for b in range(NB):
            a_v[b] = jnp.broadcast_to(h[:, b * 128:(b + 1) * 128], (H, 128)).astype(BF16)
        wait(1)
        side_step(2)
        qb = head_proj(wq_v).astype(BF16)

        wait(2)

        def uk_body(b, _):
            rows = pl.ds(pl.multiple_of(b * RB, RB), RB)
            r = jax.lax.dot_general(qb, wuk_v[rows, :], NT, preferred_element_type=F32)
            qa = jax.lax.dot_general(keep_diag(r * scale), e_v[...], NT,
                                     preferred_element_type=F32)
            a_v[b] = qa.astype(BF16)
            return 0
        jax.lax.fori_loop(0, NB, uk_body, 0)
        q_v[...] = jnp.concatenate([a_v[b] for b in range(NB)], axis=1)

        SPD = KV_DMA // KV_STEP

        def kv_body(j, carry):
            m_prev, l_prev, acc = carry

            @pl.when(j % SPD == 0)
            def _():
                i = j // SPD
                kv_copy(i).wait()

                @pl.when(i + WIN < NKV)
                def _():
                    kv_copy(i + WIN).start()

                for t in range(WIN):
                    @pl.when(i + WIN == NKV + t)
                    def _():
                        start(N_UV + t)

            for e, js in enumerate(SIDE_STEPS):
                @pl.when(j == js)
                def _():
                    side_step(3 + e)

            ck = ckv_v[pl.ds(pl.multiple_of(j * KV_STEP, KV_STEP), KV_STEP), :]
            s = jax.lax.dot_general(q_v[...], ck, NT, preferred_element_type=F32)
            m_new = jnp.maximum(m_prev, jnp.max(s, axis=1, keepdims=True))
            alpha = jnp.exp2(m_prev - m_new)
            p = jnp.exp2(s - m_new)
            l_new = l_prev * alpha + jnp.sum(p, axis=1, keepdims=True)
            acc = acc * alpha + jnp.dot(p.astype(BF16), ck, preferred_element_type=F32)
            return m_new, l_new, acc

        m0 = jnp.full((H, 1), -jnp.inf, F32)
        l0 = jnp.zeros((H, 1), F32)
        a0 = jnp.zeros((H, Dc), F32)
        _, l_fin, acc = jax.lax.fori_loop(0, Sk // KV_STEP, kv_body, (m0, l0, a0))
        o_lat = acc / l_fin

        for b in range(NB):
            a_v[b] = o_lat[:, b * 128:(b + 1) * 128].astype(BF16)
        wait(N_UV)
        ctx = head_proj(wuv_v)

        wait(N_UV + 1)
        side_step(2 * SIDE_PIECES)

        def wo_body(b, att):
            lo = jnp.concatenate(
                [jnp.where(row_h == b * HPB + j, ctx, 0.0) for j in range(HPB)], axis=1
            ).astype(BF16)
            rows = pl.ds(pl.multiple_of(b * HPB * D, HPB * D), HPB * D)
            return att + jnp.dot(lo, wo_v[rows, :], preferred_element_type=F32)
        att = jax.lax.fori_loop(0, H // HPB, wo_body, jnp.zeros((H, M), F32))
        x1 = x + ga * jnp.sum(att, axis=0, keepdims=True)

        h2 = jnp.broadcast_to((_ln(x1) * (1.0 + cb) + sb), (8, M)).astype(BF16)

        def gu_body(w, _):
            @pl.when(w == 0)
            def _():
                wait(N_UV + 2)

            @pl.when(w == 1)
            def _():
                wait(N_UV + 3)

            gu_v[w] = jnp.dot(h2, wgu_v[w], preferred_element_type=F32)
            return 0
        jax.lax.fori_loop(0, 2, gu_body, 0)
        act = _gelu(gu_v[0]) * gu_v[1]
        for i in range(F0 // WD_STEP):
            act_v[i] = act[:, i * WD_STEP:(i + 1) * WD_STEP].astype(BF16)

        for k in range((Df - F0) // VPU_STEP):
            a_k = act[0:1, F0 + k * VPU_STEP:F0 + (k + 1) * VPU_STEP].astype(BF16).astype(F32)
            acol_v[k] = jnp.broadcast_to(a_k, (128, VPU_STEP)).T

        side_step(2 * SIDE_PIECES + 1)

        def wd_body(i, ffn):
            for k, a in enumerate(wd_dmas[:WD_MXU_DMAS]):
                @pl.when(i == a // WD_STEP)
                def _():
                    wait(N_WD + k)

            rows = pl.ds(pl.multiple_of(i * WD_STEP, WD_STEP), WD_STEP)
            return ffn + jnp.dot(act_v[i], wd_v[rows, :], preferred_element_type=F32)
        ffn = jax.lax.fori_loop(0, F0 // WD_STEP, wd_body, jnp.zeros((8, M), F32))
        base = x1 + gb * ffn[0:1]

        def vpu_body(i, part):
            for k in range(WD_MXU_DMAS, len(WD_DMAS) - 1):
                @pl.when(i == (WD_DMAS[k] - F0) // VPU_STEP)
                def _():
                    wait(N_WD + k)

            rows = pl.ds(pl.multiple_of(F0 + i * VPU_STEP, VPU_STEP), VPU_STEP)
            w_i = wd_v[rows, :].astype(F32)
            a_c = acol_v[i]
            prod = jnp.concatenate(
                [w_i[:, t * 128:(t + 1) * 128] * a_c for t in range(M // 128)], axis=1)
            return part + jnp.sum(prod.reshape(VPU_STEP // 8, 8, M), axis=0)
        part = jax.lax.fori_loop(0, (Df - F0) // VPU_STEP, vpu_body, jnp.zeros((8, M), F32))
        o_ref[0] = (base + gb * jnp.sum(part, axis=0, keepdims=True)).astype(o_ref.dtype)

    hbm = pl.BlockSpec(memory_space=pl.ANY)
    return pl.pallas_call(
        kernel,
        in_specs=[hbm] * 11,
        out_specs=pl.BlockSpec(memory_space=pltpu.VMEM),
        out_shape=jax.ShapeDtypeStruct((1, Sq, M), A_x.dtype),
        scratch_shapes=[
            pltpu.VMEM((1, Sq, M), BF16),
            pltpu.VMEM((1, M), BF16),
            pltpu.VMEM((M, 6 * M), BF16),
            pltpu.VMEM((M * H, D), BF16),
            pltpu.VMEM((Dc * H, D), BF16),
            pltpu.VMEM((Sk, Dc), BF16),
            pltpu.VMEM((Dc * H, D), BF16),
            pltpu.VMEM((H * D, M), BF16),
            pltpu.VMEM((2, M, Df), BF16),
            pltpu.VMEM((Df, M), BF16),
            pltpu.VMEM((128, RB), BF16),
            pltpu.VMEM((NB, H, 128), BF16),
            pltpu.VMEM((H, Dc), BF16),
            pltpu.VMEM((2, 8, Df), F32),
            pltpu.VMEM((F0 // WD_STEP, 8, WD_STEP), BF16),
            pltpu.VMEM(((Df - F0) // VPU_STEP, VPU_STEP, 128), F32),
            pltpu.SMEM((2, SIDE_ROWS, M), BF16),
        ],
        compiler_params=pltpu.CompilerParams(vmem_limit_bytes=100 * 1024 * 1024),
    )(
        A_x, A_c_kv.reshape(Sk, Dc), A_w_q.reshape(M * H, D), A_w_uk.reshape(Dc * H, D),
        A_w_uv.reshape(Dc * H, D), A_w_o.reshape(H * D, M), B_w_gate, B_w_up, B_w_down,
        c, w_mod,
    )
```

```python
import functools
import math

import jax
import jax.numpy as jnp
import jax.experimental.pallas as pl
import jax.experimental.pallas.tpu as pltpu


F32 = jnp.float32
BF16 = jnp.bfloat16
EPS = 1e-5
NT = (((1,), (1,)), ((), ()))

KV_DMA = 1024
KV_STEP = 1024
WD_STEP = 256
WD_DMAS = (0, 768, 1280, 1408, 1536, 1664, 1728, 1792)
WD_MXU_DMAS = 2
VPU_STEP = 64
SIDE_ROWS = 288
SIDE_WO = 5
SIDE_WD = 1
SIDE_STEPS = (0, 2, 6, 11, 15, 19, 24, 28, 31)
WIN = 8


def _ln(x):
    m = jnp.mean(x, axis=-1, keepdims=True)
    d = x - m
    v = jnp.mean(d * d, axis=-1, keepdims=True)
    return d * jax.lax.rsqrt(v + EPS)


def _gelu(x):
    k = math.sqrt(2.0 / math.pi)
    return 0.5 * x * (1.0 + jnp.tanh(k * (x + 0.044715 * (x * x * x))))


@jax.jit
def pallas_adaLN_cond__compressed_kv_cla__glu_gated_geglu__decode_kernel(
    A_x: jax.Array,
    A_c_kv: jax.Array,
    A_w_q: jax.Array,
    A_w_uk: jax.Array,
    A_w_uv: jax.Array,
    A_w_o: jax.Array,
    B_x: jax.Array,
    B_w_gate: jax.Array,
    B_w_up: jax.Array,
    B_w_down: jax.Array,
    c: jax.Array,
    w_mod: jax.Array,
):
    del B_x
    _, Sq, M = A_x.shape
    _, Sk, Dc = A_c_kv.shape
    _, H, D = A_w_q.shape
    Df = B_w_gate.shape[1]
    assert (Sq, H, D) == (1, 32, 128) and M == Dc and M % 128 == 0
    assert Sk % KV_DMA == 0 and KV_DMA % KV_STEP == 0
    assert Df == WD_DMAS[-1] and all(b % WD_STEP == 0 for b in WD_DMAS[:WD_MXU_DMAS + 1])
    SIDE_PIECES = SIDE_WO + SIDE_WD
    assert SIDE_PIECES % 2 == 0 and len(SIDE_STEPS) == 2 * SIDE_PIECES - 3
    WD0 = SIDE_WD * SIDE_ROWS
    wd_dmas = (WD0,) + WD_DMAS[1:]
    assert WD0 < WD_DMAS[1] and max(SIDE_STEPS) < Sk // KV_STEP
    NKV = Sk // KV_DMA
    NB = M // 128
    RB = 128 * H
    HPB = 8
    F0 = WD_DMAS[WD_MXU_DMAS]
    scale = float(D) ** -0.5 * math.log2(math.e)

    def kernel(*refs):
        pl.run_scoped(functools.partial(body, *refs),
                      pltpu.SemaphoreType.DMA((WIN,)), pltpu.SemaphoreType.DMA((4,)))

    def body(x_hbm, ckv_hbm, wq_hbm, wuk_hbm, wuv_hbm, wo_hbm, wg_hbm, wu_hbm, wd_hbm, c_hbm,
             wmod_hbm, o_ref,
             x_v, c_v, wmod_v, wq_v, wuk_v, ckv_v, wuv_v, wo_v, wgu_v, wd_v,
             e_v, a_v, q_v, gu_v, act_v, acol_v, side_s, sem, ssem):
        pairs = [(wmod_hbm, wmod_v), (wq_hbm, wq_v), (wuk_hbm, wuk_v)]
        N_KV0 = len(pairs)
        pairs += [(ckv_hbm.at[pl.ds(i * KV_DMA, KV_DMA)], ckv_v.at[pl.ds(i * KV_DMA, KV_DMA)])
                  for i in range(NKV)]
        N_UV = len(pairs)
        wo_main = pl.ds(SIDE_WO * SIDE_ROWS, H * D - SIDE_WO * SIDE_ROWS)
        pairs += [(wuv_hbm, wuv_v), (wo_hbm.at[wo_main], wo_v.at[wo_main]),
                  (wg_hbm, wgu_v.at[0]), (wu_hbm, wgu_v.at[1])]
        N_WD = len(pairs)
        pairs += [(wd_hbm.at[pl.ds(a, b - a)], wd_v.at[pl.ds(a, b - a)])
                  for a, b in zip(wd_dmas[:-1], wd_dmas[1:])]

        def copy(n):
            return pltpu.make_async_copy(pairs[n][0], pairs[n][1], sem.at[n % WIN])

        def start(n):
            if n < len(pairs):
                copy(n).start()

        def wait(n):
            copy(n).wait()
            start(n + WIN)

        def kv_copy(i):
            rows = pl.ds(pl.multiple_of(i * KV_DMA, KV_DMA), KV_DMA)
            return pltpu.make_async_copy(ckv_hbm.at[rows], ckv_v.at[rows],
                                         sem.at[(N_KV0 + i) % WIN])

        def side(e):
            k = (e // 4) * 2 + e % 2
            src, dst, k0 = (wo_hbm, wo_v, 0) if k < SIDE_WO else (wd_hbm, wd_v, SIDE_WO)
            rows = pl.ds((k - k0) * SIDE_ROWS, SIDE_ROWS)
            if e % 4 < 2:
                return pltpu.make_async_copy(src.at[rows], side_s.at[k % 2], ssem.at[e % 4])
            return pltpu.make_async_copy(side_s.at[k % 2], dst.at[rows], ssem.at[e % 4])

        def side_step(e):
            side(e - 2).wait()
            if e < 2 * SIDE_PIECES:
                side(e).start()

        cp_c = pltpu.make_async_copy(c_hbm, c_v, sem.at[0])
        cp_x = pltpu.make_async_copy(x_hbm, x_v, sem.at[0])
        start(0)
        cp_c.start()
        cp_x.start()
        for n in range(1, WIN):
            start(n)
        side(0).start()
        side(1).start()

        r_i = jax.lax.broadcasted_iota(jnp.int32, (128, RB), 0)
        n_i = jax.lax.broadcasted_iota(jnp.int32, (128, RB), 1)
        e_v[...] = jnp.where(r_i == n_i // H, 1.0, 0.0).astype(BF16)

        row_h = jax.lax.broadcasted_iota(jnp.int32, (H, 128), 0)
        diag = row_h == (jax.lax.broadcasted_iota(jnp.int32, (H, 128), 1) % H)

        def keep_diag(r):
            return jnp.concatenate(
                [jnp.where(diag, r[:, t * 128:(t + 1) * 128], 0.0) for t in range(RB // 128)],
                axis=1).astype(BF16)

        def head_proj(w_v):
            def body(b, out):
                rep = jnp.dot(a_v[b], e_v[...], preferred_element_type=F32)
                rows = pl.ds(pl.multiple_of(b * RB, RB), RB)
                return out + jnp.dot(keep_diag(rep), w_v[rows, :], preferred_element_type=F32)
            return jax.lax.fori_loop(0, NB, body, jnp.zeros((H, D), F32))

        copy(0).wait()
        cp_c.wait()
        cp_x.wait()
        start(WIN)
        cf = c_v[...].astype(F32)
        sc = (cf * jax.nn.sigmoid(cf)).astype(BF16)
        mod = jnp.dot(sc, wmod_v[...], preferred_element_type=F32)
        sa, ca, ga, sb, cb, gb = [mod[:, i * M:(i + 1) * M] for i in range(6)]
        x = x_v[0].astype(F32)
        h = _ln(x) * (1.0 + ca) + sa

        for b in range(NB):
            a_v[b] = jnp.broadcast_to(h[:, b * 128:(b + 1) * 128], (H, 128)).astype(BF16)
        wait(1)
        side_step(2)
        qb = head_proj(wq_v).astype(BF16)

        wait(2)

        def uk_body(b, _):
            rows = pl.ds(pl.multiple_of(b * RB, RB), RB)
            r = jax.lax.dot_general(qb, wuk_v[rows, :], NT, preferred_element_type=F32)
            qa = jax.lax.dot_general(keep_diag(r * scale), e_v[...], NT,
                                     preferred_element_type=F32)
            a_v[b] = qa.astype(BF16)
            return 0
        jax.lax.fori_loop(0, NB, uk_body, 0)
        q_v[...] = jnp.concatenate([a_v[b] for b in range(NB)], axis=1)

        SPD = KV_DMA // KV_STEP

        def kv_body(j, carry):
            m_prev, l_prev, acc = carry

            @pl.when(j % SPD == 0)
            def _():
                i = j // SPD
                kv_copy(i).wait()

                @pl.when(i + WIN < NKV)
                def _():
                    kv_copy(i + WIN).start()

                for t in range(WIN):
                    @pl.when(i + WIN == NKV + t)
                    def _():
                        start(N_UV + t)

            for e, js in enumerate(SIDE_STEPS):
                @pl.when(j == js)
                def _():
                    side_step(3 + e)

            ck = ckv_v[pl.ds(pl.multiple_of(j * KV_STEP, KV_STEP), KV_STEP), :]
            s = jax.lax.dot_general(q_v[...], ck, NT, preferred_element_type=F32)
            m_new = jnp.maximum(m_prev, jnp.max(s, axis=1, keepdims=True))
            alpha = jnp.exp2(m_prev - m_new)
            p = jnp.exp2(s - m_new)
            l_new = l_prev * alpha + jnp.sum(p, axis=1, keepdims=True)
            acc = acc * alpha + jnp.dot(p.astype(BF16), ck, preferred_element_type=F32)
            return m_new, l_new, acc

        m0 = jnp.full((H, 1), -jnp.inf, F32)
        l0 = jnp.zeros((H, 1), F32)
        a0 = jnp.zeros((H, Dc), F32)
        _, l_fin, acc = jax.lax.fori_loop(0, Sk // KV_STEP, kv_body, (m0, l0, a0))
        o_lat = acc / l_fin

        for b in range(NB):
            a_v[b] = o_lat[:, b * 128:(b + 1) * 128].astype(BF16)
        wait(N_UV)
        ctx = head_proj(wuv_v)

        wait(N_UV + 1)
        side_step(2 * SIDE_PIECES)

        def wo_body(b, att):
            lo = jnp.concatenate(
                [jnp.where(row_h == b * HPB + j, ctx, 0.0) for j in range(HPB)], axis=1
            ).astype(BF16)
            rows = pl.ds(pl.multiple_of(b * HPB * D, HPB * D), HPB * D)
            return att + jnp.dot(lo, wo_v[rows, :], preferred_element_type=F32)
        att = jax.lax.fori_loop(0, H // HPB, wo_body, jnp.zeros((H, M), F32))
        x1 = x + ga * jnp.sum(att, axis=0, keepdims=True)

        h2 = jnp.broadcast_to((_ln(x1) * (1.0 + cb) + sb), (8, M)).astype(BF16)

        def gu_body(w, _):
            @pl.when(w == 0)
            def _():
                wait(N_UV + 2)

            @pl.when(w == 1)
            def _():
                wait(N_UV + 3)

            gu_v[w] = jnp.dot(h2, wgu_v[w], preferred_element_type=F32)
            return 0
        jax.lax.fori_loop(0, 2, gu_body, 0)
        act = _gelu(gu_v[0]) * gu_v[1]
        for i in range(F0 // WD_STEP):
            act_v[i] = act[:, i * WD_STEP:(i + 1) * WD_STEP].astype(BF16)

        for k in range((Df - F0) // VPU_STEP):
            a_k = act[0:1, F0 + k * VPU_STEP:F0 + (k + 1) * VPU_STEP].astype(BF16).astype(F32)
            acol_v[k] = jnp.broadcast_to(a_k, (128, VPU_STEP)).T

        side_step(2 * SIDE_PIECES + 1)

        def wd_body(i, ffn):
            for k, a in enumerate(wd_dmas[:WD_MXU_DMAS]):
                @pl.when(i == a // WD_STEP)
                def _():
                    wait(N_WD + k)

            rows = pl.ds(pl.multiple_of(i * WD_STEP, WD_STEP), WD_STEP)
            return ffn + jnp.dot(act_v[i], wd_v[rows, :], preferred_element_type=F32)
        ffn = jax.lax.fori_loop(0, F0 // WD_STEP, wd_body, jnp.zeros((8, M), F32))
        base = x1 + gb * ffn[0:1]

        def vpu_body(i, part):
            for k in range(WD_MXU_DMAS, len(WD_DMAS) - 1):
                @pl.when(i == (WD_DMAS[k] - F0) // VPU_STEP)
                def _():
                    wait(N_WD + k)

            rows = pl.ds(pl.multiple_of(F0 + i * VPU_STEP, VPU_STEP), VPU_STEP)
            w_i = wd_v[rows, :].astype(F32)
            a_c = acol_v[i]
            prod = jnp.concatenate(
                [w_i[:, t * 128:(t + 1) * 128] * a_c for t in range(M // 128)], axis=1)
            return part + jnp.sum(prod.reshape(VPU_STEP // 8, 8, M), axis=0)
        part = jax.lax.fori_loop(0, (Df - F0) // VPU_STEP, vpu_body, jnp.zeros((8, M), F32))
        o_ref[0] = (base + gb * jnp.sum(part, axis=0, keepdims=True)).astype(o_ref.dtype)

    hbm = pl.BlockSpec(memory_space=pl.ANY)
    return pl.pallas_call(
        kernel,
        in_specs=[hbm] * 11,
        out_specs=pl.BlockSpec(memory_space=pltpu.VMEM),
        out_shape=jax.ShapeDtypeStruct((1, Sq, M), A_x.dtype),
        scratch_shapes=[
            pltpu.VMEM((1, Sq, M), BF16),
            pltpu.VMEM((1, M), BF16),
            pltpu.VMEM((M, 6 * M), BF16),
            pltpu.VMEM((M * H, D), BF16),
            pltpu.VMEM((Dc * H, D), BF16),
            pltpu.VMEM((Sk, Dc), BF16),
            pltpu.VMEM((Dc * H, D), BF16),
            pltpu.VMEM((H * D, M), BF16),
            pltpu.VMEM((2, M, Df), BF16),
            pltpu.VMEM((Df, M), BF16),
            pltpu.VMEM((128, RB), BF16),
            pltpu.VMEM((NB, H, 128), BF16),
            pltpu.VMEM((H, Dc), BF16),
            pltpu.VMEM((2, 8, Df), F32),
            pltpu.VMEM((F0 // WD_STEP, 8, WD_STEP), BF16),
            pltpu.VMEM(((Df - F0) // VPU_STEP, VPU_STEP, 128), F32),
            pltpu.SMEM((2, SIDE_ROWS, M), BF16),
        ],
        compiler_params=pltpu.CompilerParams(vmem_limit_bytes=100 * 1024 * 1024),
    )(
        A_x, A_c_kv.reshape(Sk, Dc), A_w_q.reshape(M * H, D), A_w_uk.reshape(Dc * H, D),
        A_w_uv.reshape(Dc * H, D), A_w_o.reshape(H * D, M), B_w_gate, B_w_up, B_w_down,
        c, w_mod,
    )
```
